```python
import jax
import jax.numpy as jnp

def _softmax(x, axis=-1):
    return jax.nn.softmax(x, axis=axis)

def _gelu(x):
    return jax.nn.gelu(x, approximate=True)

def _silu(x):
    return jax.nn.silu(x)

def _sigmoid(x):
    return jax.nn.sigmoid(x)

def _layernorm(x, axis=-1, eps=1e-05):
    m = jnp.mean(x, axis=axis, keepdims=True)
    v = jnp.var(x, axis=axis, keepdims=True)
    return (x - m) / jnp.sqrt(v + eps)

def _scatter_add(tgt, idx, src, axis=0):
    return tgt.at[idx].add(src)

def _segment_sum(src, seg, n):
    return jax.ops.segment_sum(src, seg, n)

class _Rng:

    def __init__(self, key):
        self._k = key

    def _next(self):
        self._k, sub = jax.random.split(self._k)
        return sub

    def normal(self, shape):
        return jax.random.normal(self._next(), shape, dtype=jnp.bfloat16)

    def randint(self, lo, hi, shape):
        return jax.random.randint(self._next(), shape, lo, hi, dtype=jnp.int32)

    def uniform(self, shape, lo=0.0, hi=1.0):
        return jax.random.uniform(self._next(), shape, jnp.bfloat16, lo, hi)

    def permutation(self, n):
        return jax.random.permutation(self._next(), n)
kernel_name = 'concat_heads__softmax_full_mha__memory_aug_recurrent_mem_tr__prompt'

def setup_inputs():
    _rng = _Rng(jax.random.key(int.from_bytes(__import__("os").urandom(4), "little")))
    _w = lambda a: (lambda t: t.astype(jnp.bfloat16) if jnp.issubdtype(t.dtype, jnp.floating) else t)(jnp.asarray(a))

    def _A_setup():
        B, S, D = (1, 2048, 1024)
        return {'x': _w((lambda *s: _rng.normal(s) * 0.05)(B, S, D)), 'wqkv': _w((lambda *s: _rng.normal(s) * 0.05)(D, 3 * D)), 'wo': _w((lambda *s: _rng.normal(s) * 0.05)(D, D))}
    _A_in = _A_setup()

    def _B_setup():
        B, S, Dm = (1, 2048, 1024)
        H, Dh = (32, 128)
        M, seg = (8, 32)
        seg = min(seg, S)
        S = S // seg * seg
        return {'x': _w((lambda *s: _rng.normal(s) * 0.05)(B, S, Dm)), 'mem0': _w((lambda *s: _rng.normal(s) * 0.05)(B, M, Dm)), 'Wq': _w((lambda *s: _rng.normal(s) * 0.05)(Dm, H, Dh) * Dm ** (-0.5)), 'Wk': _w((lambda *s: _rng.normal(s) * 0.05)(Dm, H, Dh) * Dm ** (-0.5)), 'Wv': _w((lambda *s: _rng.normal(s) * 0.05)(Dm, H, Dh) * Dm ** (-0.5)), 'Wo': _w((lambda *s: _rng.normal(s) * 0.05)(H, Dh, Dm) * (H * Dh) ** (-0.5)), 'seg_len': seg}
    _B_in = _B_setup()
    return {'A_x': _A_in['x'], 'A_wqkv': _A_in['wqkv'], 'A_wo': _A_in['wo'], 'B_x': _B_in['x'], 'B_mem0': _B_in['mem0'], 'B_Wq': _B_in['Wq'], 'B_Wk': _B_in['Wk'], 'B_Wv': _B_in['Wv'], 'B_Wo': _B_in['Wo'], 'B_seg_len': _B_in['seg_len']}

def reference(A_x, A_wqkv, A_wo, B_x, B_mem0, B_Wq, B_Wk, B_Wv, B_Wo, B_seg_len):

    def _A_ref(x, wqkv, wo):
        B, S, D = x.shape
        H = 32
        Dh = D // H
        qkv = (lambda x, *d: x.transpose(*d))((x @ wqkv).reshape(B, S, 3, H, Dh), 2, 0, 3, 1, 4)
        q, k, v = (qkv[0], qkv[1], qkv[2])
        scale = Dh ** (-0.5)
        scores = jnp.einsum('bhqd,bhkd->bhqk', q, k) * scale
        p = _softmax(scores, axis=-1)
        o = jnp.einsum('bhqk,bhkd->bhqd', p, v)
        return (lambda x, *d: x.transpose(*d))(o, 0, 2, 1, 3).reshape(B, S, D) @ wo

    def _B_ref(x, mem0, Wq, Wk, Wv, Wo, seg_len):
        B, S, Dm = x.shape
        H, Dh = (Wq.shape[1], Wq.shape[2])
        M = mem0.shape[1]
        scale = Dh ** (-0.5)
        n_seg = S // seg_len
        L = M + seg_len
        idx = jnp.arange(L)
        mask = (idx[:, None] < M) | (idx[:, None] >= idx[None, :])
        mem = mem0
        outs = []
        for s in range(n_seg):
            xs = x[:, s * seg_len:(s + 1) * seg_len, :].copy()
            h = jnp.concatenate([mem, xs], axis=1)
            q = jnp.einsum('btd,dhe->bhte', h, Wq)
            k = jnp.einsum('btd,dhe->bhte', h, Wk)
            v = jnp.einsum('btd,dhe->bhte', h, Wv)
            scores = jnp.einsum('bhqe,bhke->bhqk', q, k) * scale
            scores = jnp.where(mask[None, None], scores, -1000000000.0)
            p = _softmax(scores, axis=-1)
            o = jnp.einsum('bhqk,bhke->bhqe', p, v)
            o = jnp.einsum('bhte,hed->btd', o, Wo)
            mem = o[:, :M, :].copy()
            outs.append(o[:, M:, :])
        return jnp.concatenate(outs, axis=1)
    a = _A_ref(A_x, A_wqkv, A_wo)
    b = _B_ref(B_x, B_mem0, B_Wq, B_Wk, B_Wv, B_Wo, B_seg_len)
    return jnp.concatenate([a, b], axis=-1)
```

```python
import functools

import jax
import jax.numpy as jnp
import numpy as np
from jax import lax
from jax.experimental import pallas as pl
from jax.experimental.pallas import tpu as pltpu

f32 = jnp.float32
bf16 = jnp.bfloat16
u32 = jnp.uint32

LOG2E = 1.4426950408889634

S = 2048
D = 1024
HA = 32
DHA = D // HA
HB = 32
DHB = 128
M = 8
SEG = 32
L = M + SEG
NSEG = S // SEG

NQ = 512
NQB = S // NQ
KT = 128
NKT = S // KT
NCHUNK = HA * NQB
CPS = NCHUNK // NSEG
RB = 512
NRB = S // RB
NSTAGE = 8


def _pk(x):
    return pltpu.bitcast(x, u32)


def _upk(x):
    return pltpu.bitcast(x, bf16)


def _kernel(ax_hbm, wqkv_hbm, awo_hbm, bx_hbm, mem0_hbm, wq_hbm, wk_hbm, wv_hbm, wo_hbm,
            out_hbm,
            xa, wqkv, awo, k4, q4, vt, ot, xb, mem0v, stage, wp, wop, h_ref, o_ref, qm_ref,
            sem_in, sem_stage, sem_oa, sem_ob, *s_refs):
    sb = [s_refs[0:NKT], s_refs[NKT:2 * NKT]]

    def x_copy(rb):
        return pltpu.make_async_copy(ax_hbm.at[pl.ds(rb * RB, RB), :], xa.at[pl.ds(rb * RB, RB), :],
                                     sem_in.at[rb])

    def w_copy(j):
        return pltpu.make_async_copy(wqkv_hbm.at[:, pl.ds(j * D, D)], wqkv.at[:, pl.ds(j * D, D)],
                                     sem_in.at[NRB + j])

    awo_copy = pltpu.make_async_copy(awo_hbm, awo, sem_in.at[NRB + 3])
    xb_copy = pltpu.make_async_copy(bx_hbm, xb, sem_in.at[NRB + 4])
    mem_copy = pltpu.make_async_copy(mem0_hbm, mem0v, sem_in.at[NRB + 5])
    wo32 = wo_hbm.bitcast(u32)

    def wo_copy(n):
        return pltpu.make_async_copy(wo32.at[:, pl.ds(n * 128, 128)], wop.at[n], sem_in.at[NRB + 6 + n])

    wb32 = [w.bitcast(u32) for w in (wq_hbm, wk_hbm, wv_hbm)]

    def stage_copy(i):
        hp, j = divmod(i, 3)
        slot = i % NSTAGE
        return pltpu.make_async_copy(wb32[j].at[:, hp, :], stage.at[slot], sem_stage.at[slot])

    def repack(i):
        hp, j = divmod(i, 3)
        slot = i % NSTAGE
        x = stage[slot]
        lo = pltpu.bitcast(x << 16, f32).astype(bf16)
        hi = pltpu.bitcast(x & jnp.uint32(0xFFFF0000), f32).astype(bf16)
        wp[j * HB + 2 * hp] = _pk(lo)
        wp[j * HB + 2 * hp + 1] = _pk(hi)

    NSLAB = 3 * HB // 2
    slab_state = {"next_start": 0, "next_done": 0}

    def slabs_start(n):
        for _ in range(n):
            if slab_state["next_start"] < NSLAB:
                stage_copy(slab_state["next_start"]).start()
                slab_state["next_start"] += 1

    def slabs_process(n):
        for _ in range(n):
            i = slab_state["next_done"]
            if i < NSLAB:
                stage_copy(i).wait()
                repack(i)
                slab_state["next_done"] += 1
                slabs_start(1)

    w_copy(1).start()
    x_copy(0).start()
    w_copy(1).wait()
    x_copy(0).wait()
    for rb in range(1, NRB):
        x_copy(rb).start()
    w_copy(0).start()
    w_copy(2).start()
    slabs_start(NSTAGE)

    def proj_nat(j, rb, dst, scale):
        xs = xa[rb * RB:(rb + 1) * RB, :]
        for g in range(8):
            r = jnp.dot(xs, wqkv[:, j * D + g * 128: j * D + (g + 1) * 128], preferred_element_type=f32)
            if scale is not None:
                r = r * scale
            dst[g, rb * RB // 2:(rb + 1) * RB // 2, :] = _pk(r.astype(bf16))

    def proj_t(j, rb, dst):
        xs = xa[rb * RB:(rb + 1) * RB, :]
        r = lax.dot_general(wqkv[:, j * D:(j + 1) * D], xs, (((0,), (1,)), ((), ())),
                            preferred_element_type=f32)
        dst[:, rb * RB:(rb + 1) * RB] = _pk(r.astype(bf16))

    slabs_per_piece = NSLAB // (3 * NRB)
    for rb in range(NRB):
        if rb > 0:
            x_copy(rb).wait()
        proj_nat(1, rb, k4, None)
        slabs_process(slabs_per_piece)
    w_copy(0).wait()
    for n in range(8):
        wo_copy(n).start()
    for rb in range(NRB):
        proj_nat(0, rb, q4, (DHA ** -0.5) * LOG2E)
        slabs_process(slabs_per_piece)
    w_copy(2).wait()
    xb_copy.start()
    mem_copy.start()
    for rb in range(NRB):
        proj_t(2, rb, vt)
        slabs_process(slabs_per_piece)
    awo_copy.start()
    for n in range(8):
        wo_copy(n).wait()
    xb_copy.wait()
    mem_copy.wait()

    lane = lax.broadcasted_iota(jnp.int32, (NQ // 2, 128), 1)

    def prep_q(ci):
        hh = ci // NQB
        qb = ci % NQB
        g = hh // 4
        hl = hh % 4
        q0 = pl.multiple_of(qb * (NQ // 2), NQ // 2)
        qq = q4[g, pl.ds(q0, NQ // 2), :]
        qm_ref[...] = jnp.where((lane >= hl * DHA) & (lane < hl * DHA + DHA), qq, jnp.zeros_like(qq))

    def qk_piece(ci, kt, sbuf, mx):
        g = (ci // NQB) // 4
        kk = _upk(k4[g, kt * KT // 2:(kt + 1) * KT // 2, :])
        qm = _upk(qm_ref[...])
        st = lax.dot_general(kk, qm, (((1,), (1,)), ((), ())), preferred_element_type=f32)
        sbuf[kt][...] = st
        pm = jnp.max(st.reshape(KT // 8, 8, NQ), axis=0)
        return pm if mx is None else jnp.maximum(mx, pm)

    def sm_piece(ci, kt, sbuf, m, l, acc):
        hh = ci // NQB
        p = jnp.exp2(sbuf[kt][...] - m)
        ps = jnp.sum(p.reshape(KT // 8, 8, NQ), axis=0)
        l = ps if l is None else l + ps
        h0 = pl.multiple_of(hh * (DHA // 2), DHA // 2)
        vv = _upk(vt[pl.ds(h0, DHA // 2), kt * KT:(kt + 1) * KT])
        d = jnp.dot(vv, p.astype(bf16), preferred_element_type=f32)
        acc = d if acc is None else acc + d
        return l, acc

    def a_finish(ci, l, acc):
        hh = ci // NQB
        qb = ci % NQB
        lt = jnp.sum(l, axis=0, keepdims=True)
        o = (acc * pltpu.reciprocal(lt, approx=False)).astype(bf16)
        h0 = pl.multiple_of(hh * (DHA // 2), DHA // 2)
        q0 = pl.multiple_of(qb * NQ, NQ)
        ot[pl.ds(h0, DHA // 2), pl.ds(q0, NQ)] = _pk(o)

    def a_gen(s, m, last):
        for j in range(CPS):
            ci = s * CPS + j
            has_next = not (last and j == CPS - 1)
            cur, nxt = sb[j % 2], sb[(j + 1) % 2]
            if has_next:
                prep_q(ci + 1)
            mx = l = acc = None
            for kt in range(NKT):
                if has_next:
                    mx = qk_piece(ci + 1, kt, nxt, mx)
                l, acc = sm_piece(ci, kt, cur, m, l, acc)
                if kt == NKT - 1:
                    a_finish(ci, l, acc)
                    if has_next:
                        m = jnp.max(mx, axis=0, keepdims=True)
                yield m

    cb = (DHB ** -0.5) * LOG2E
    row = lax.broadcasted_iota(jnp.int32, (L, L), 0)
    col = lax.broadcasted_iota(jnp.int32, (L, L), 1)
    mask = (row < M) | (row >= col)
    KSPLIT = 24 * DHB
    D1, D2 = 1, 1

    def ob_copy(r0):
        return pltpu.make_async_copy(xb.at[pl.ds(r0, SEG), :], out_hbm.at[pl.ds(r0, SEG), pl.ds(D, D)], sem_ob)

    def step(s, m, last=False):
        r0 = pl.multiple_of(s * SEG, SEG)
        h_ref[M:L, :] = xb[pl.ds(r0, SEG), :].astype(f32)
        ag = a_gen(s, m, last)
        npieces = CPS * NKT
        done = 0
        st = {}
        for t in range(HB + D1 + D2):
            if t < HB:
                hs = h_ref[...]
                q = jnp.dot(hs, _upk(wp[t]), preferred_element_type=f32) * cb
                k = jnp.dot(hs, _upk(wp[HB + t]), preferred_element_type=f32)
                v = jnp.dot(hs, _upk(wp[2 * HB + t]), preferred_element_type=f32)
                st[t] = dict(q=q, k=k.astype(bf16), v=v.astype(bf16))
            hd = t - D1
            if 0 <= hd < HB:
                e = st[hd]
                sc = lax.dot_general(e["q"], e["k"], (((1,), (1,)), ((), ())), preferred_element_type=f32)
                sc = jnp.where(mask, sc, -1e9 * LOG2E)
                mm = jnp.max(sc, axis=1, keepdims=True)
                p = jnp.exp2(sc - mm)
                e["p"] = p
                e["r"] = pltpu.reciprocal(jnp.sum(p, axis=1, keepdims=True), approx=False)
            hd = t - D1 - D2
            if 0 <= hd < HB:
                e = st.pop(hd)
                o = jnp.dot(e["p"], e["v"], preferred_element_type=f32) * e["r"]
                o_ref[:, hd * DHB:(hd + 1) * DHB] = o
            while done < min(npieces, (t + 1) * npieces // HB):
                m = next(ag)
                done += 1
        o1 = o_ref[:, :KSPLIT]
        parts = [jnp.dot(o1, _upk(wop[n, :KSPLIT // 2, :]), preferred_element_type=f32) for n in range(8)]
        o2 = o_ref[:, KSPLIT:]
        for n in range(8):
            r = parts[n] + jnp.dot(o2, _upk(wop[n, KSPLIT // 2:, :]), preferred_element_type=f32)
            ob = r.astype(bf16)
            xb[pl.ds(r0, SEG), n * 128:(n + 1) * 128] = ob[M:L]
            h_ref[0:M, n * 128:(n + 1) * 128] = ob[0:M].astype(f32)
        ob_copy(r0).start()
        return m

    h_ref[0:M, :] = mem0v[...].astype(f32)
    prep_q(0)
    mx = None
    for kt in range(NKT):
        mx = qk_piece(0, kt, sb[0], mx)
    m0 = jnp.max(mx, axis=0, keepdims=True)

    m_fin = lax.fori_loop(0, NSEG - 1, step, m0)
    step(NSEG - 1, m_fin, last=True)

    awo_copy.wait()

    def oa_copy(rb):
        return pltpu.make_async_copy(xa.at[pl.ds(rb * RB, RB), :], out_hbm.at[pl.ds(rb * RB, RB), pl.ds(0, D)],
                                     sem_oa.at[rb])

    for rb in range(NRB):
        o_t = _upk(ot[:, rb * RB:(rb + 1) * RB])
        r = lax.dot_general(o_t, awo[...], (((0,), (0,)), ((), ())), preferred_element_type=f32)
        xa[rb * RB:(rb + 1) * RB, :] = r.astype(bf16)
        oa_copy(rb).start()
    for rb in range(NRB):
        oa_copy(rb).wait()
    pltpu.make_async_copy(xb, out_hbm.at[:, pl.ds(D, D)], sem_ob).wait()


@functools.partial(jax.jit, static_argnames=("B_seg_len",))
def pallas_concat_heads__softmax_full_mha__memory_aug_recurrent_mem_tr__prompt_kernel(
    A_x: jax.Array,
    A_wqkv: jax.Array,
    A_wo: jax.Array,
    B_x: jax.Array,
    B_mem0: jax.Array,
    B_Wq: jax.Array,
    B_Wk: jax.Array,
    B_Wv: jax.Array,
    B_Wo: jax.Array,
    B_seg_len: int = SEG,
):
    assert A_x.shape == (1, S, D) and B_x.shape == (1, S, D) and B_mem0.shape == (1, M, D)
    assert B_Wq.shape == (D, HB, DHB) and B_Wo.shape == (HB, DHB, D)
    assert int(B_seg_len) == SEG

    scratch = [
        pltpu.VMEM((S, D), bf16),
        pltpu.VMEM((D, 3 * D), bf16),
        pltpu.VMEM((D, D), bf16),
        pltpu.VMEM((8, S // 2, 128), u32),
        pltpu.VMEM((8, S // 2, 128), u32),
        pltpu.VMEM((D // 2, S), u32),
        pltpu.VMEM((D // 2, S), u32),
        pltpu.VMEM((S, D), bf16),
        pltpu.VMEM((M, D), bf16),
        pltpu.VMEM((NSTAGE, D, 128), u32),
        pltpu.VMEM((3 * HB, D // 2, 128), u32),
        pltpu.VMEM((8, HB * DHB // 2, 128), u32),
        pltpu.VMEM((L, D), f32),
        pltpu.VMEM((L, HB * DHB), f32),
        pltpu.VMEM((NQ // 2, 128), u32),
        pltpu.SemaphoreType.DMA((NRB + 6 + 8,)),
        pltpu.SemaphoreType.DMA((NSTAGE,)),
        pltpu.SemaphoreType.DMA((NRB,)),
        pltpu.SemaphoreType.DMA,
    ] + [pltpu.VMEM((KT, NQ), f32)] * (2 * NKT)

    out = pl.pallas_call(
        _kernel,
        out_shape=jax.ShapeDtypeStruct((S, 2 * D), bf16),
        in_specs=[pl.BlockSpec(memory_space=pl.ANY)] * 9,
        out_specs=pl.BlockSpec(memory_space=pl.ANY),
        scratch_shapes=scratch,
        compiler_params=pltpu.CompilerParams(vmem_limit_bytes=112 * 1024 * 1024),
    )(A_x.reshape(S, D), A_wqkv, A_wo, B_x.reshape(S, D), B_mem0.reshape(M, D), B_Wq, B_Wk, B_Wv,
      B_Wo.reshape(HB * DHB, D))
    return out.reshape(1, S, 2 * D)
```

```python
import functools, contextlib

import jax
import jax.numpy as jnp
import numpy as np
from jax import lax
from jax.experimental import pallas as pl
from jax.experimental.pallas import tpu as pltpu

CFG = dict(tok=1,rsub=64,pm=256,rtok=1,vt2=2,unroll=2,aslots=36)
f32 = jnp.float32
bf16 = jnp.bfloat16
u32 = jnp.uint32

LOG2E = 1.4426950408889634

S = 2048
D = 1024
HA = 32
DHA = D // HA
HB = 32
DHB = 128
M = 8
SEG = 32
L = M + SEG
NSEG = S // SEG

NQ = 512
NQB = S // NQ
KT = 128
NKT = S // KT
NCHUNK = HA * NQB
CPS = NCHUNK // NSEG
RB = 512
NRB = S // RB
NSTAGE = 20


def _pk(x):
    return pltpu.bitcast(x, u32)


def _upk(x):
    return pltpu.bitcast(x, bf16)


def _kernel(ax_hbm, wqkv_hbm, awo_hbm, bx_hbm, mem0_hbm, wq_hbm, wk_hbm, wv_hbm, wo_hbm,
            out_hbm,
            xa, wqkv, awo, k4, q4, vt, ot, xb, mem0v, stage, wp, wop, h_ref, o_ref, qm_ref, wvt,
            sem_in, sem_stage, sem_oa, sem_ob, *s_refs):
    sb = [s_refs[0:NKT], s_refs[NKT:2 * NKT]]

    def x_copy(rb):
        return pltpu.make_async_copy(ax_hbm.at[pl.ds(rb * RB, RB), :], xa.at[pl.ds(rb * RB, RB), :],
                                     sem_in.at[rb])

    awo_copy = pltpu.make_async_copy(awo_hbm, awo, sem_in.at[NRB + 3])
    mem_copy = pltpu.make_async_copy(mem0_hbm, mem0v, sem_in.at[NRB + 5])
    wo32 = wo_hbm.bitcast(u32)

    def wo_copy(n):
        return pltpu.make_async_copy(wo32.at[:, pl.ds(n * 128, 128)], wop.at[n], sem_in.at[NRB + 6 + n])

    wb32 = [w.bitcast(u32) for w in (wq_hbm, wk_hbm, wv_hbm)]

    class _Multi:
        def __init__(self, cps):
            self.cps = cps

        def start(self):
            for c in self.cps:
                c.start()

        def wait(self):
            for c in self.cps:
                c.wait()

    def stage_copy(i):
        hp, j = divmod(i, 3)
        slot = i % NSTAGE
        if CFG.get("eo", "stride") == "stride":
            return pltpu.make_async_copy(wb32[j].at[:, hp, :], stage.at[slot], sem_stage.at[slot])
        return _Multi([pltpu.make_async_copy(wb32[j].at[:, par, hp, :], stage.at[slot, par], sem_stage.at[slot])
                       for par in range(2)])

    tokq = []

    def attach_tok(y):
        if not tokq:
            return y
        t = tokq.pop()
        while tokq:
            t = jnp.maximum(t, tokq.pop())
        yi = pltpu.bitcast(y[0:8], jnp.int32)
        y0 = pltpu.bitcast(jnp.minimum(yi, jnp.maximum(yi, t)), u32)
        return jnp.concatenate([y0, y[8:]], axis=0)

    RSUB = CFG.get("rsub", 128)

    def repack_gen(i):
        hp, j = divmod(i, 3)
        slot = i % NSTAGE
        for r in range(0, D // 2, RSUB // 2):
            n = RSUB // 2
            if CFG.get("eo", "stride") == "stride":
                e = stage[slot, pl.ds(2 * r, n, stride=2), :]
                o = stage[slot, pl.ds(2 * r + 1, n, stride=2), :]
            else:
                e = stage[slot, 0, r:r + n, :]
                o = stage[slot, 1, r:r + n, :]
            lo = (e & jnp.uint32(0xFFFF)) | (o << 16)
            hi = (e >> 16) | (o & jnp.uint32(0xFFFF0000))
            wp[j * HB + 2 * hp, r:r + n, :] = lo
            wp[j * HB + 2 * hp + 1, r:r + n, :] = hi
            if CFG.get("rtok", 0):
                t = jnp.maximum(pltpu.bitcast(lo, jnp.int32), pltpu.bitcast(hi, jnp.int32))
                t = jnp.max(t.reshape(n // 8, 8, 128), axis=0)
                tokq.append(t)
            yield

    NSLAB = 3 * HB // 2

    PM = CFG.get("pm", 512)

    def proj_nat(j, rb, dst, scale):
        for r in range(rb * RB, (rb + 1) * RB, PM):
            xs = xa[r:r + PM, :]
            for g in range(8):
                y = jnp.dot(xs, wqkv[:, j * D + g * 128: j * D + (g + 1) * 128], preferred_element_type=f32)
                if scale is not None:
                    y = y * scale
                dst[g, r // 2:(r + PM) // 2, :] = attach_tok(_pk(y.astype(bf16)))
                yield

    def proj_t(j, rb, dst):
        for r in range(rb * RB, (rb + 1) * RB, 128):
            xs = xa[r:r + 128, :]
            y = lax.dot_general(wqkv[:, j * D:(j + 1) * D], xs, (((0,), (1,)), ((), ())),
                                preferred_element_type=f32)
            dst[:, r:r + 128] = _pk(y.astype(bf16))
            yield

    TM = CFG.get("tm", 256)

    def proj_t3(rb, dst):
        if rb == 0:
            wvt[...] = wqkv[:, 2 * D:3 * D].T
        for r in range(rb * RB, (rb + 1) * RB, 128):
            xs = xa[r:r + 128, :]
            for n0 in range(0, D, TM):
                y = lax.dot_general(wvt[n0:n0 + TM, :], xs, (((1,), (1,)), ((), ())), preferred_element_type=f32)
                dst[n0 // 2:(n0 + TM) // 2, r:r + 128] = attach_tok(_pk(y.astype(bf16)))
                yield

    def proj_t2(j, rb, dst):
        for r in range(rb * RB, (rb + 1) * RB, PM):
            xs = xa[r:r + PM, :]
            for g in range(8):
                y = jnp.dot(xs, wqkv[:, j * D + g * 128: j * D + (g + 1) * 128], preferred_element_type=f32)
                yt = _pk(y.astype(bf16).T)
                dst[g * 64:(g + 1) * 64, r:r + 128] = attach_tok(yt[:, 0:128])
                if PM > 128:
                    dst[g * 64:(g + 1) * 64, r + 128:r + PM] = yt[:, 128:]
                yield

    GROUPS = CFG.get("groups", (2, 8, 8, 10, 10, 10))
    GOFF = [sum(GROUPS[:i]) for i in range(len(GROUPS) + 1)]
    assert GOFF[-1] == NSLAB and max(GROUPS[i] + GROUPS[i + 1] for i in range(len(GROUPS) - 1)) <= NSTAGE

    def slab_group_start(g):
        for i in range(GOFF[g], GOFF[g + 1]):
            stage_copy(i).start()

    def slab_group_wait(g):
        for i in range(GOFF[g], GOFF[g + 1]):
            stage_copy(i).wait()

    def slab_group_repack(g):
        for i in range(GOFF[g], GOFF[g + 1]):
            yield from repack_gen(i)

    def interleave(main, side, n_main, n_side):
        done = 0
        for i in range(n_main):
            next(main)
            while done < (i + 1) * n_side // n_main:
                next(side)
                done += 1

    NPIECE = 3 * NRB

    def wq_half(j, hf):
        return pltpu.make_async_copy(wqkv_hbm.at[pl.ds(hf * (D // 2), D // 2), pl.ds(j * D, D)],
                                     wqkv.at[pl.ds(hf * (D // 2), D // 2), pl.ds(j * D, D)],
                                     sem_in.at[NRB + 6 + 8 + j * 2 + hf])

    def xb_copy(c):
        return pltpu.make_async_copy(bx_hbm.at[pl.ds(c * RB, RB), :], xb.at[pl.ds(c * RB, RB), :],
                                     sem_in.at[NRB + 6 + 8 + 6 + c])

    class _G:
        def __init__(self, g):
            self.g = g

        def start(self):
            slab_group_start(self.g)

        def wait(self):
            slab_group_wait(self.g)

    starts = {
        -1: [wq_half(1, 0), x_copy(0), wq_half(1, 1)],
        0: [x_copy(1), x_copy(2), x_copy(3), _G(0)],
        1: [_G(1)],
        2: [wq_half(0, 0), wq_half(0, 1), _G(2)],
        4: [wq_half(2, 0), wq_half(2, 1), _G(3)],
        6: [_G(4)] + [wo_copy(n) for n in range(0, 2)],
        8: [_G(5)] + [wo_copy(n) for n in range(2, 4)],
        10: [mem_copy, xb_copy(0)] + [wo_copy(n) for n in range(4, 8)],
        12: [xb_copy(c) for c in range(1, NRB)] + ([awo_copy] if CFG.get('stop') != 'pro' else []),
    }
    waits = {
        0: [wq_half(1, 0), x_copy(0), wq_half(1, 1)],
        1: [x_copy(1), x_copy(2), x_copy(3), _G(0)],
        2: [_G(1)],
        4: [wq_half(0, 0), wq_half(0, 1), _G(2)],
        6: [wq_half(2, 0), wq_half(2, 1), _G(3)],
        8: [_G(4)] + [wo_copy(n) for n in range(0, 2)],
        10: [_G(5)] + [wo_copy(n) for n in range(2, 4)],
        12: [mem_copy, xb_copy(0)] + [wo_copy(n) for n in range(4, 8)],
    }
    repack_at = {1: (0, 1), 2: (1, 2), 4: (2, 2), 6: (3, 2), 8: (4, 2), 10: (5, 2)}
    for c in starts[-1]:
        c.start()
    side, side_left, pieces_left = iter(()), 0, 0
    for p in range(NPIECE + 1):
        j, rb = divmod(p, NRB)
        if CFG.get("scopes"):
            with jax.named_scope(f"wait_{p:02d}"):
                for c in waits.get(p, []):
                    c.wait()
        else:
            for c in waits.get(p, []):
                c.wait()
        for c in starts.get(p, []):
            c.start()
        if p == NPIECE:
            break
        if p in repack_at:
            assert side_left == 0
            g, pieces_left = repack_at[p]
            side, side_left = slab_group_repack(g), GROUPS[g] * D // RSUB
        n_side = side_left // pieces_left if pieces_left else 0
        side_left -= n_side
        pieces_left = max(pieces_left - 1, 0)
        if j == 0:
            main, n_main = proj_nat(1, rb, k4, None), 8 * RB // PM
        elif j == 1:
            main, n_main = proj_nat(0, rb, q4, (DHA ** -0.5) * LOG2E), 8 * RB // PM
        elif CFG.get("vt2", 1) == 1:
            main, n_main = proj_t2(2, rb, vt), 8 * RB // PM
        elif CFG.get("vt2", 1) == 2:
            main, n_main = proj_t3(rb, vt), RB // 128 * (D // TM)
        else:
            main, n_main = proj_t(2, rb, vt), RB // 128
        interleave(main, side, n_main, n_side)
    assert side_left == 0

    lane = lax.broadcasted_iota(jnp.int32, (NQ // 2, 128), 1)

    def prep_q(ci):
        hh = ci // NQB
        qb = ci % NQB
        g = hh // 4
        hl = hh % 4
        q0 = pl.multiple_of(qb * (NQ // 2), NQ // 2)
        qq = q4[g, pl.ds(q0, NQ // 2), :]
        qm_ref[...] = jnp.where((lane >= hl * DHA) & (lane < hl * DHA + DHA), qq, jnp.zeros_like(qq))

    def qk_piece(ci, kt, sbuf, mx):
        g = (ci // NQB) // 4
        kk = _upk(k4[g, kt * KT // 2:(kt + 1) * KT // 2, :])
        qm = _upk(qm_ref[...])
        st = lax.dot_general(kk, qm, (((1,), (1,)), ((), ())), preferred_element_type=f32)
        sbuf[kt][...] = st
        pm = jnp.max(st.reshape(KT // 8, 8, NQ), axis=0)
        return pm if mx is None else jnp.maximum(mx, pm)

    def sm_piece(ci, kt, sbuf, m, l, acc, tok=None):
        hh = ci // NQB
        if tok is not None and CFG.get("tok", 0):
            m = jnp.minimum(m, jnp.maximum(m, tok))
        p = jnp.exp2(sbuf[kt][...] - m)
        ps = jnp.sum(p.reshape(KT // 8, 8, NQ), axis=0)
        l = ps if l is None else l + ps
        h0 = pl.multiple_of(hh * (DHA // 2), DHA // 2)
        vv = _upk(vt[pl.ds(h0, DHA // 2), kt * KT:(kt + 1) * KT])
        d = jnp.dot(vv, p.astype(bf16), preferred_element_type=f32)
        acc = d if acc is None else acc + d
        return l, acc

    def recip_a(x):
        if CFG.get("fastrcp", 1):
            r = pltpu.reciprocal(x, approx=True)
            return r * (2.0 - x * r)
        return pltpu.reciprocal(x, approx=False)

    def a_finish(ci, l, acc):
        hh = ci // NQB
        qb = ci % NQB
        lt = jnp.sum(l, axis=0, keepdims=True)
        o = (acc * recip_a(lt)).astype(bf16)
        h0 = pl.multiple_of(hh * (DHA // 2), DHA // 2)
        q0 = pl.multiple_of(qb * NQ, NQ)
        ot[pl.ds(h0, DHA // 2), pl.ds(q0, NQ)] = _pk(o)

    def a_gen(s, m, last):
        for j in range(CPS):
            ci = s * CPS + j
            has_next = not (last and j == CPS - 1)
            cur, nxt = sb[j % 2], sb[(j + 1) % 2]
            if has_next:
                prep_q(ci + 1)
            mx = l = acc = None
            toks = []
            for kt in range(NKT):
                if has_next:
                    mx = qk_piece(ci + 1, kt, nxt, mx)
                    toks.append(mx)
                lag = CFG.get("toklag", 1)
                tok = toks[kt - lag] if (has_next and kt - lag >= 0) else None
                if tok is not None:
                    tok = tok[0:1]
                l, acc = sm_piece(ci, kt, cur, m, l, acc, tok)
                if kt == NKT - 1:
                    a_finish(ci, l, acc)
                    if has_next:
                        m = jnp.max(mx, axis=0, keepdims=True)
                yield m

    cb = (DHB ** -0.5) * LOG2E
    row = lax.broadcasted_iota(jnp.int32, (L, L), 0)
    col = lax.broadcasted_iota(jnp.int32, (L, L), 1)
    mask = (row < M) | (row >= col)
    KSPLIT = CFG.get('ksplit', 24) * DHB
    D1, D2 = CFG.get('d1', 1), CFG.get('d2', 1)

    def ob_copy(r0):
        return pltpu.make_async_copy(xb.at[pl.ds(r0, SEG), :], out_hbm.at[pl.ds(r0, SEG), pl.ds(D, D)], sem_ob)

    def recip(x):
        if CFG.get("fastrcp", 1):
            r = pltpu.reciprocal(x, approx=True)
            return r * (2.0 - x * r)
        return pltpu.reciprocal(x, approx=False)

    def step(s, m, last=False):
        r0 = s * SEG if isinstance(s, int) else pl.multiple_of(s * SEG, SEG)
        h_ref[M:L, :] = xb[pl.ds(r0, SEG), :].astype(f32)
        ag = a_gen(s, m, last)
        npieces = CPS * NKT
        state = dict(done=0, m=m)
        st = {}
        nslots = HB + D1 + D2
        aslots = CFG.get("aslots", nslots)

        def a_upto(n):
            while state["done"] < min(npieces, n):
                state["m"] = next(ag)
                state["done"] += 1

        parts = {}
        o1 = {}

        def p3a(n):
            if "v" not in o1:
                o1["v"] = o_ref[:, :KSPLIT]
            parts[n] = jnp.dot(o1["v"], _upk(wop[n, :KSPLIT // 2, :]), preferred_element_type=f32)

        p3a_sched = CFG.get("p3a", {32: [0, 1, 2, 3], 33: [4, 5, 6, 7]})
        for t in range(nslots):
            if t < HB:
                hs = h_ref[...]
                q = jnp.dot(hs, _upk(wp[t]), preferred_element_type=f32) * cb
                k = jnp.dot(hs, _upk(wp[HB + t]), preferred_element_type=f32)
                v = jnp.dot(hs, _upk(wp[2 * HB + t]), preferred_element_type=f32)
                st[t] = dict(q=q, k=k.astype(bf16), v=v.astype(bf16))
            hd = t - D1
            if 0 <= hd < HB:
                e = st[hd]
                sc = lax.dot_general(e["q"], e["k"], (((1,), (1,)), ((), ())), preferred_element_type=f32)
                sc = jnp.where(mask, sc, -1e9 * LOG2E)
                mm = jnp.max(sc, axis=1, keepdims=True)
                p = jnp.exp2(sc - mm)
                e["p"] = p
                e["r"] = recip(jnp.sum(p, axis=1, keepdims=True))
            hd = t - D1 - D2
            if 0 <= hd < HB:
                e = st.pop(hd)
                o = jnp.dot(e["p"], e["v"], preferred_element_type=f32) * e["r"]
                o_ref[:, hd * DHB:(hd + 1) * DHB] = o
            a_upto((t + 1) * npieces // aslots)
            for n in p3a_sched.get(t, []):
                p3a(n)
        for n in range(8):
            if n not in parts:
                p3a(n)
        o2 = o_ref[:, KSPLIT:]
        for n in range(8):
            r = parts[n] + jnp.dot(o2, _upk(wop[n, KSPLIT // 2:, :]), preferred_element_type=f32)
            ob = r.astype(bf16)
            xb[pl.ds(r0, SEG), n * 128:(n + 1) * 128] = ob[M:L]
            h_ref[0:M, n * 128:(n + 1) * 128] = ob[0:M].astype(f32)
        a_upto(npieces)
        ob_copy(r0).start()
        return state["m"]

    h_ref[0:M, :] = mem0v[...].astype(f32)
    prep_q(0)
    mx = None
    for kt in range(NKT):
        mx = qk_piece(0, kt, sb[0], mx)
    m0 = jnp.max(mx, axis=0, keepdims=True)

    if CFG.get("stop") == "pro":
        ot[0:8, 0:NQ] = pltpu.bitcast(jnp.broadcast_to(m0, (8, NQ)), u32)
        return
    SPC = RB // SEG

    def chunk_wait(c):
        pltpu.make_async_copy(bx_hbm.at[pl.ds(0, RB), :], xb.at[pl.ds(0, RB), :],
                              sem_in.at[NRB + 6 + 8 + 6 + c]).wait()

    UN = CFG.get("unroll", 1)
    if UN == 2:
        def step2(i, m):
            @pl.when((i % (SPC // 2) == 0) & (i > 0))
            def _():
                chunk_wait(i // (SPC // 2))
            m = step(2 * i, m)
            return step(2 * i + 1, m)

        m_fin = lax.fori_loop(0, NSEG // 2 - 1, step2, m0)
        m_fin = step(NSEG - 2, m_fin)
    elif CFG.get("nested", 1):
        def outer(c, m):
            @pl.when(c > 0)
            def _():
                chunk_wait(c)
            n = jnp.where(c == NRB - 1, SPC - 1, SPC)
            return lax.fori_loop(0, n, lambda i, mm: step(c * SPC + i, mm), m)

        m_fin = lax.fori_loop(0, NRB, outer, m0)
    else:
        def step_w(s, m):
            @pl.when((s % SPC == 0) & (s > 0))
            def _():
                chunk_wait(s // SPC)
            return step(s, m)

        m_fin = lax.fori_loop(0, NSEG - 1, step_w, m0)
    step(NSEG - 1, m_fin, last=True)

    awo_copy.wait()

    def oa_copy(rb):
        return pltpu.make_async_copy(xa.at[pl.ds(rb * RB, RB), :], out_hbm.at[pl.ds(rb * RB, RB), pl.ds(0, D)],
                                     sem_oa.at[rb])

    for rb in range(NRB):
        o_t = _upk(ot[:, rb * RB:(rb + 1) * RB])
        r = lax.dot_general(o_t, awo[...], (((0,), (0,)), ((), ())), preferred_element_type=f32)
        xa[rb * RB:(rb + 1) * RB, :] = r.astype(bf16)
        oa_copy(rb).start()
    with jax.named_scope("final_waits") if CFG.get("scopes") else contextlib.nullcontext():
        for rb in range(NRB):
            oa_copy(rb).wait()
    if CFG.get("nsteps", NSEG) == NSEG:
        pltpu.make_async_copy(xb, out_hbm.at[:, pl.ds(D, D)], sem_ob).wait()
    else:
        n = CFG["nsteps"] * SEG
        pltpu.make_async_copy(xb.at[pl.ds(0, n), :], out_hbm.at[pl.ds(0, n), pl.ds(D, D)], sem_ob).wait()


@functools.partial(jax.jit, static_argnames=("B_seg_len",))
def pallas_concat_heads__softmax_full_mha__memory_aug_recurrent_mem_tr__prompt_kernel(
    A_x: jax.Array,
    A_wqkv: jax.Array,
    A_wo: jax.Array,
    B_x: jax.Array,
    B_mem0: jax.Array,
    B_Wq: jax.Array,
    B_Wk: jax.Array,
    B_Wv: jax.Array,
    B_Wo: jax.Array,
    B_seg_len: int = SEG,
):
    assert A_x.shape == (1, S, D) and B_x.shape == (1, S, D) and B_mem0.shape == (1, M, D)
    assert B_Wq.shape == (D, HB, DHB) and B_Wo.shape == (HB, DHB, D)
    assert int(B_seg_len) == SEG

    scratch = [
        pltpu.VMEM((S, D), bf16),
        pltpu.VMEM((D, 3 * D), bf16),
        pltpu.VMEM((D, D), bf16),
        pltpu.VMEM((8, S // 2, 128), u32),
        pltpu.VMEM((8, S // 2, 128), u32),
        pltpu.VMEM((D // 2, S), u32),
        pltpu.VMEM((D // 2, S), u32),
        pltpu.VMEM((S, D), bf16),
        pltpu.VMEM((M, D), bf16),
        (pltpu.VMEM((NSTAGE, D, 128), u32) if CFG.get('eo','stride')=='stride' else pltpu.VMEM((NSTAGE, 2, D // 2, 128), u32)),
        pltpu.VMEM((3 * HB, D // 2, 128), u32),
        pltpu.VMEM((8, HB * DHB // 2, 128), u32),
        pltpu.VMEM((L, D), f32),
        pltpu.VMEM((L, HB * DHB), f32),
        pltpu.VMEM((NQ // 2, 128), u32),
        pltpu.VMEM((D, D), bf16),
        pltpu.SemaphoreType.DMA((NRB + 6 + 8 + 6 + NRB,)),
        pltpu.SemaphoreType.DMA((NSTAGE,)),
        pltpu.SemaphoreType.DMA((NRB,)),
        pltpu.SemaphoreType.DMA,
    ] + [pltpu.VMEM((KT, NQ), f32)] * (2 * NKT)

    out = pl.pallas_call(
        _kernel,
        out_shape=jax.ShapeDtypeStruct((S, 2 * D), bf16),
        in_specs=[pl.BlockSpec(memory_space=pl.ANY)] * 9,
        out_specs=pl.BlockSpec(memory_space=pl.ANY),
        scratch_shapes=scratch,
        compiler_params=pltpu.CompilerParams(vmem_limit_bytes=112 * 1024 * 1024),
    )(A_x.reshape(S, D), A_wqkv, A_wo, B_x.reshape(S, D), B_mem0.reshape(M, D), *[(w if CFG.get('eo','stride')=='stride' else w.reshape(D // 2, 2, HB, DHB)) for w in (B_Wq, B_Wk, B_Wv)],
      B_Wo.reshape(HB * DHB, D))
    return out.reshape(1, S, 2 * D)
```

```python
import functools, contextlib

import jax
import jax.numpy as jnp
import numpy as np
from jax import lax
from jax.experimental import pallas as pl
from jax.experimental.pallas import tpu as pltpu

CFG = dict(rsub=64,pm=256,rtok=1,vt2=2,tok=1,toklag=2,pstore=1,nested=0,d1=1,d2=2,aslots=35,p3a={31:[0],32:[1,2],33:[3,4,5],34:[6,7]},afirst_from=33,qk0_early=1,groups=(1,7,10,10,10,10),oblocks=(512,512,512,256,256))
f32 = jnp.float32
bf16 = jnp.bfloat16
u32 = jnp.uint32

LOG2E = 1.4426950408889634

S = 2048
D = 1024
HA = 32
DHA = D // HA
HB = 32
DHB = 128
M = 8
SEG = 32
L = M + SEG
NSEG = S // SEG

NQ = 512
NQB = S // NQ
KT = 128
NKT = S // KT
NCHUNK = HA * NQB
CPS = NCHUNK // NSEG
RB = 512
NRB = S // RB
NSTAGE = 20


def _pk(x):
    return pltpu.bitcast(x, u32)


def _upk(x):
    return pltpu.bitcast(x, bf16)


def _kernel(ax_hbm, wqkv_hbm, awo_hbm, bx_hbm, mem0_hbm, wq_hbm, wk_hbm, wv_hbm, wo_hbm,
            out_hbm,
            xa, wqkv, awo, k4, q4, vt, ot, xb, mem0v, stage, wp, wop, h_ref, o_ref, qm_ref, wvt, part_ref,
            sem_in, sem_stage, sem_oa, sem_ob, *s_refs):
    sb = [s_refs[0:NKT], s_refs[NKT:2 * NKT]]

    def x_copy(rb):
        return pltpu.make_async_copy(ax_hbm.at[pl.ds(rb * RB, RB), :], xa.at[pl.ds(rb * RB, RB), :],
                                     sem_in.at[rb])

    awo_copy = pltpu.make_async_copy(awo_hbm, awo, sem_in.at[NRB + 3])
    mem_copy = pltpu.make_async_copy(mem0_hbm, mem0v, sem_in.at[NRB + 5])
    wo32 = wo_hbm.bitcast(u32)

    def wo_copy(n):
        return pltpu.make_async_copy(wo32.at[:, pl.ds(n * 128, 128)], wop.at[n], sem_in.at[NRB + 6 + n])

    wb32 = [w.bitcast(u32) for w in (wq_hbm, wk_hbm, wv_hbm)]

    class _Multi:
        def __init__(self, cps):
            self.cps = cps

        def start(self):
            for c in self.cps:
                c.start()

        def wait(self):
            for c in self.cps:
                c.wait()

    def stage_copy(i):
        hp, j = divmod(i, 3)
        slot = i % NSTAGE
        if CFG.get("eo", "stride") == "stride":
            return pltpu.make_async_copy(wb32[j].at[:, hp, :], stage.at[slot], sem_stage.at[slot])
        return _Multi([pltpu.make_async_copy(wb32[j].at[:, par, hp, :], stage.at[slot, par], sem_stage.at[slot])
                       for par in range(2)])

    tokq = []

    def attach_tok(y):
        if not tokq:
            return y
        t = tokq.pop()
        while tokq:
            t = jnp.maximum(t, tokq.pop())
        yi = pltpu.bitcast(y[0:8], jnp.int32)
        y0 = pltpu.bitcast(jnp.minimum(yi, jnp.maximum(yi, t)), u32)
        return jnp.concatenate([y0, y[8:]], axis=0)

    RSUB = CFG.get("rsub", 128)

    def repack_gen(i):
        hp, j = divmod(i, 3)
        slot = i % NSTAGE
        for r in range(0, D // 2, RSUB // 2):
            n = RSUB // 2
            if CFG.get("eo", "stride") == "stride":
                e = stage[slot, pl.ds(2 * r, n, stride=2), :]
                o = stage[slot, pl.ds(2 * r + 1, n, stride=2), :]
            else:
                e = stage[slot, 0, r:r + n, :]
                o = stage[slot, 1, r:r + n, :]
            lo = (e & jnp.uint32(0xFFFF)) | (o << 16)
            hi = (e >> 16) | (o & jnp.uint32(0xFFFF0000))
            wp[j * HB + 2 * hp, r:r + n, :] = lo
            wp[j * HB + 2 * hp + 1, r:r + n, :] = hi
            if CFG.get("rtok", 0):
                t = jnp.maximum(pltpu.bitcast(lo, jnp.int32), pltpu.bitcast(hi, jnp.int32))
                t = jnp.max(t.reshape(n // 8, 8, 128), axis=0)
                tokq.append(t)
            yield

    NSLAB = 3 * HB // 2

    PM = CFG.get("pm", 512)

    def proj_nat(j, rb, dst, scale):
        for r in range(rb * RB, (rb + 1) * RB, PM):
            xs = xa[r:r + PM, :]
            for g in range(8):
                y = jnp.dot(xs, wqkv[:, j * D + g * 128: j * D + (g + 1) * 128], preferred_element_type=f32)
                if scale is not None:
                    y = y * scale
                dst[g, r // 2:(r + PM) // 2, :] = attach_tok(_pk(y.astype(bf16)))
                yield

    def proj_t(j, rb, dst):
        for r in range(rb * RB, (rb + 1) * RB, 128):
            xs = xa[r:r + 128, :]
            y = lax.dot_general(wqkv[:, j * D:(j + 1) * D], xs, (((0,), (1,)), ((), ())),
                                preferred_element_type=f32)
            dst[:, r:r + 128] = _pk(y.astype(bf16))
            yield

    TM = CFG.get("tm", 256)

    def proj_t3(rb, dst):
        if rb == 0:
            wvt[...] = wqkv[:, 2 * D:3 * D].T
        for r in range(rb * RB, (rb + 1) * RB, 128):
            xs = xa[r:r + 128, :]
            for n0 in range(0, D, TM):
                y = lax.dot_general(wvt[n0:n0 + TM, :], xs, (((1,), (1,)), ((), ())), preferred_element_type=f32)
                dst[n0 // 2:(n0 + TM) // 2, r:r + 128] = attach_tok(_pk(y.astype(bf16)))
                yield

    def proj_t2(j, rb, dst):
        for r in range(rb * RB, (rb + 1) * RB, PM):
            xs = xa[r:r + PM, :]
            for g in range(8):
                y = jnp.dot(xs, wqkv[:, j * D + g * 128: j * D + (g + 1) * 128], preferred_element_type=f32)
                yt = _pk(y.astype(bf16).T)
                dst[g * 64:(g + 1) * 64, r:r + 128] = attach_tok(yt[:, 0:128])
                if PM > 128:
                    dst[g * 64:(g + 1) * 64, r + 128:r + PM] = yt[:, 128:]
                yield

    GROUPS = CFG.get("groups", (2, 8, 8, 10, 10, 10))
    GOFF = [sum(GROUPS[:i]) for i in range(len(GROUPS) + 1)]
    assert GOFF[-1] == NSLAB and max(GROUPS[i] + GROUPS[i + 1] for i in range(len(GROUPS) - 1)) <= NSTAGE

    def slab_group_start(g):
        for i in range(GOFF[g], GOFF[g + 1]):
            stage_copy(i).start()

    def slab_group_wait(g):
        for i in range(GOFF[g], GOFF[g + 1]):
            stage_copy(i).wait()

    def slab_group_repack(g):
        for i in range(GOFF[g], GOFF[g + 1]):
            yield from repack_gen(i)

    def interleave(main, side, n_main, n_side):
        done = 0
        for i in range(n_main):
            next(main)
            while done < (i + 1) * n_side // n_main:
                next(side)
                done += 1

    NPIECE = 3 * NRB

    def wq_half(j, hf):
        return pltpu.make_async_copy(wqkv_hbm.at[pl.ds(hf * (D // 2), D // 2), pl.ds(j * D, D)],
                                     wqkv.at[pl.ds(hf * (D // 2), D // 2), pl.ds(j * D, D)],
                                     sem_in.at[NRB + 6 + 8 + j * 2 + hf])

    def xb_copy(c):
        return pltpu.make_async_copy(bx_hbm.at[pl.ds(c * RB, RB), :], xb.at[pl.ds(c * RB, RB), :],
                                     sem_in.at[NRB + 6 + 8 + 6 + c])

    class _G:
        def __init__(self, g):
            self.g = g

        def start(self):
            slab_group_start(self.g)

        def wait(self):
            slab_group_wait(self.g)

    starts = {
        -1: [wq_half(1, 0), x_copy(0), wq_half(1, 1)],
        0: [x_copy(1), x_copy(2), x_copy(3), _G(0)],
        1: [_G(1)],
        2: [wq_half(0, 0), wq_half(0, 1), _G(2)],
        4: [wq_half(2, 0), wq_half(2, 1), _G(3)],
        6: [_G(4)] + [wo_copy(n) for n in range(0, 2)],
        8: [_G(5)] + [wo_copy(n) for n in range(2, 4)],
        10: [mem_copy, xb_copy(0)] + [wo_copy(n) for n in range(4, 8)],
        12: [xb_copy(c) for c in range(1, NRB)] + ([awo_copy] if CFG.get('stop') != 'pro' else []),
    }
    waits = {
        0: [wq_half(1, 0), x_copy(0), wq_half(1, 1)],
        1: [x_copy(1), x_copy(2), x_copy(3), _G(0)],
        2: [_G(1)],
        4: [wq_half(0, 0), wq_half(0, 1), _G(2)],
        6: [wq_half(2, 0), wq_half(2, 1), _G(3)],
        8: [_G(4)] + [wo_copy(n) for n in range(0, 2)],
        10: [_G(5)] + [wo_copy(n) for n in range(2, 4)],
        12: [mem_copy, xb_copy(0)] + [wo_copy(n) for n in range(4, 8)],
    }
    repack_at = {1: (0, 1), 2: (1, 2), 4: (2, 2), 6: (3, 2), 8: (4, 2), 10: (5, 2)}
    lane = lax.broadcasted_iota(jnp.int32, (NQ // 2, 128), 1)

    def prep_q(ci):
        hh = ci // NQB
        qb = ci % NQB
        g = hh // 4
        hl = hh % 4
        q0 = pl.multiple_of(qb * (NQ // 2), NQ // 2)
        qq = q4[g, pl.ds(q0, NQ // 2), :]
        qm_ref[...] = jnp.where((lane >= hl * DHA) & (lane < hl * DHA + DHA), qq, jnp.zeros_like(qq))

    def qk_piece(ci, kt, sbuf, mx):
        g = (ci // NQB) // 4
        kk = _upk(k4[g, kt * KT // 2:(kt + 1) * KT // 2, :])
        qm = _upk(qm_ref[...])
        st = lax.dot_general(kk, qm, (((1,), (1,)), ((), ())), preferred_element_type=f32)
        sbuf[kt][...] = st
        pm = jnp.max(st.reshape(KT // 8, 8, NQ), axis=0)
        return pm if mx is None else jnp.maximum(mx, pm)

    def sm_piece(ci, kt, sbuf, m, l, acc, tok=None):
        hh = ci // NQB
        if tok is not None and CFG.get("tok", 0):
            mi = pltpu.bitcast(m, jnp.int32)
            m = pltpu.bitcast(jnp.minimum(mi, jnp.maximum(mi, pltpu.bitcast(tok, jnp.int32))), f32)
        p = jnp.exp2(sbuf[kt][...] - m)
        ps = jnp.sum(p.reshape(KT // 8, 8, NQ), axis=0)
        l = ps if l is None else l + ps
        h0 = pl.multiple_of(hh * (DHA // 2), DHA // 2)
        vv = _upk(vt[pl.ds(h0, DHA // 2), kt * KT:(kt + 1) * KT])
        d = jnp.dot(vv, p.astype(bf16), preferred_element_type=f32)
        acc = d if acc is None else acc + d
        return l, acc

    def recip_a(x):
        if CFG.get("fastrcp", 1):
            r = pltpu.reciprocal(x, approx=True)
            return r * (2.0 - x * r)
        return pltpu.reciprocal(x, approx=False)

    def a_finish(ci, l, acc):
        hh = ci // NQB
        qb = ci % NQB
        lt = jnp.sum(l, axis=0, keepdims=True)
        o = (acc * recip_a(lt)).astype(bf16)
        h0 = pl.multiple_of(hh * (DHA // 2), DHA // 2)
        q0 = pl.multiple_of(qb * NQ, NQ)
        ot[pl.ds(h0, DHA // 2), pl.ds(q0, NQ)] = _pk(o)

    def first_scores():
        prep_q(0)
        mx = None
        for kt in range(NKT):
            mx = qk_piece(0, kt, sb[0], mx)
        return jnp.max(mx, axis=0, keepdims=True)

    for c in starts[-1]:
        c.start()
    side, side_left, pieces_left = iter(()), 0, 0
    for p in range(NPIECE + 1):
        j, rb = divmod(p, NRB)
        if CFG.get("scopes"):
            with jax.named_scope(f"wait_{p:02d}"):
                for c in waits.get(p, []):
                    c.wait()
        else:
            for c in waits.get(p, []):
                c.wait()
        for c in starts.get(p, []):
            c.start()
        if p == NPIECE:
            break
        if p == CFG.get("qk0_at", 8) and CFG.get("qk0_early"):
            pass
        if p in repack_at:
            assert side_left == 0
            g, pieces_left = repack_at[p]
            side, side_left = slab_group_repack(g), GROUPS[g] * D // RSUB
        n_side = side_left // pieces_left if pieces_left else 0
        side_left -= n_side
        pieces_left = max(pieces_left - 1, 0)
        if j == 0:
            main, n_main = proj_nat(1, rb, k4, None), 8 * RB // PM
        elif j == 1:
            main, n_main = proj_nat(0, rb, q4, (DHA ** -0.5) * LOG2E), 8 * RB // PM
        elif CFG.get("vt2", 1) == 1:
            main, n_main = proj_t2(2, rb, vt), 8 * RB // PM
        elif CFG.get("vt2", 1) == 2:
            main, n_main = proj_t3(rb, vt), RB // 128 * (D // TM)
        else:
            main, n_main = proj_t(2, rb, vt), RB // 128
        interleave(main, side, n_main, n_side)
        if CFG.get("qk0_early") and p == 7:
            m0 = first_scores()
    assert side_left == 0

    def a_gen(s, m, last):
        for j in range(CPS):
            ci = s * CPS + j
            has_next = not (last and j == CPS - 1)
            cur, nxt = sb[j % 2], sb[(j + 1) % 2]
            if has_next:
                prep_q(ci + 1)
            mx = l = acc = None
            toks = []
            for kt in range(NKT):
                if has_next:
                    mx = qk_piece(ci + 1, kt, nxt, mx)
                    toks.append(mx)
                lag = CFG.get("toklag", 1)
                tok = toks[kt - lag] if (has_next and kt - lag >= 0) else None
                if tok is not None:
                    tok = tok[0:1]
                l, acc = sm_piece(ci, kt, cur, m, l, acc, tok)
                if kt == NKT - 1:
                    a_finish(ci, l, acc)
                    if has_next:
                        m = jnp.max(mx, axis=0, keepdims=True)
                yield m

    cb = (DHB ** -0.5) * LOG2E
    row = lax.broadcasted_iota(jnp.int32, (L, L), 0)
    col = lax.broadcasted_iota(jnp.int32, (L, L), 1)
    mask = (row < M) | (row >= col)
    KSPLIT = CFG.get('ksplit', 24) * DHB
    D1, D2 = CFG.get('d1', 1), CFG.get('d2', 1)

    def ob_copy(r0):
        return pltpu.make_async_copy(xb.at[pl.ds(r0, SEG), :], out_hbm.at[pl.ds(r0, SEG), pl.ds(D, D)], sem_ob)

    def recip(x):
        if CFG.get("fastrcp", 1):
            r = pltpu.reciprocal(x, approx=True)
            return r * (2.0 - x * r)
        return pltpu.reciprocal(x, approx=False)

    def step(s, m, last=False):
        r0 = s * SEG if isinstance(s, int) else pl.multiple_of(s * SEG, SEG)
        h_ref[M:L, :] = xb[pl.ds(r0, SEG), :].astype(f32)
        R0 = M if (last and CFG.get("deadrows", 1)) else 0
        ag = a_gen(s, m, last)
        npieces = CPS * NKT
        state = dict(done=0, m=m)
        st = {}
        nslots = HB + D1 + D2
        aslots = CFG.get("aslots", nslots)

        def a_upto(n):
            while state["done"] < min(npieces, n):
                state["m"] = next(ag)
                state["done"] += 1

        parts = {}
        o1 = {}

        def p3a(n):
            if "v" not in o1:
                o1["v"] = o_ref[R0:L, :KSPLIT]
            parts[n] = jnp.dot(o1["v"], _upk(wop[n, :KSPLIT // 2, :]), preferred_element_type=f32)
            if CFG.get("pstore"):
                part_ref[n, R0:L] = parts[n]
                parts[n] = None

        p3a_sched = CFG.get("p3a", {32: [0, 1, 2, 3], 33: [4, 5, 6, 7]})
        for t in range(nslots):
            if t >= CFG.get("afirst_from", 99):
                a_upto((t + 1) * npieces // aslots)
            if t < HB:
                hs = h_ref[...]
                q = jnp.dot(h_ref[R0:L, :] if R0 else hs, _upk(wp[t]), preferred_element_type=f32) * cb
                k = jnp.dot(hs, _upk(wp[HB + t]), preferred_element_type=f32)
                v = jnp.dot(hs, _upk(wp[2 * HB + t]), preferred_element_type=f32)
                st[t] = dict(q=q, k=k.astype(bf16), v=v.astype(bf16))
            hd = t - D1
            if 0 <= hd < HB:
                e = st[hd]
                sc = lax.dot_general(e["q"], e["k"], (((1,), (1,)), ((), ())), preferred_element_type=f32)
                sc = jnp.where(mask[R0:L], sc, -1e9 * LOG2E)
                mm = jnp.max(sc, axis=1, keepdims=True)
                p = jnp.exp2(sc - mm)
                e["p"] = p
                e["r"] = recip(jnp.sum(p, axis=1, keepdims=True))
            hd = t - D1 - D2
            if 0 <= hd < HB:
                e = st.pop(hd)
                o = jnp.dot(e["p"], e["v"], preferred_element_type=f32) * e["r"]
                o_ref[R0:L, hd * DHB:(hd + 1) * DHB] = o
            a_upto((t + 1) * npieces // aslots)
            for n in p3a_sched.get(t, []):
                p3a(n)
        for n in range(8):
            if n not in parts:
                p3a(n)
        o2 = o_ref[R0:L, KSPLIT:]
        for n in range(8):
            pn = parts[n] if parts[n] is not None else part_ref[n, R0:L]
            r = pn + jnp.dot(o2, _upk(wop[n, KSPLIT // 2:, :]), preferred_element_type=f32)
            ob = r.astype(bf16)
            if R0:
                xb[pl.ds(r0, SEG), n * 128:(n + 1) * 128] = ob
            else:
                xb[pl.ds(r0, SEG), n * 128:(n + 1) * 128] = ob[M:L]
                h_ref[0:M, n * 128:(n + 1) * 128] = ob[0:M].astype(f32)
        a_upto(npieces)
        ob_copy(r0).start()
        return state["m"]

    h_ref[0:M, :] = mem0v[...].astype(f32)
    if not CFG.get("qk0_early"):
        m0 = first_scores()

    if CFG.get("stop") == "pro":
        ot[0:8, 0:NQ] = pltpu.bitcast(jnp.broadcast_to(m0, (8, NQ)), u32)
        return
    SPC = RB // SEG

    def chunk_wait(c):
        c0 = pl.multiple_of(c * RB, RB)
        pltpu.make_async_copy(bx_hbm.at[pl.ds(c0, RB), :], xb.at[pl.ds(c0, RB), :],
                              sem_in.at[NRB + 6 + 8 + 6 + c]).wait()

    UN = CFG.get("unroll", 1)
    if UN == 2:
        def step2(i, m):
            @pl.when((i % (SPC // 2) == 0) & (i > 0))
            def _():
                chunk_wait(i // (SPC // 2))
            m = step(2 * i, m)
            return step(2 * i + 1, m)

        m_fin = lax.fori_loop(0, NSEG // 2 - 1, step2, m0)
        m_fin = step(NSEG - 2, m_fin)
    elif CFG.get("nested", 1):
        def outer(c, m):
            @pl.when(c > 0)
            def _():
                chunk_wait(c)
            n = jnp.where(c == NRB - 1, SPC - 1, SPC)
            return lax.fori_loop(0, n, lambda i, mm: step(c * SPC + i, mm), m)

        m_fin = lax.fori_loop(0, NRB, outer, m0)
    else:
        def step_w(s, m):
            @pl.when((s % SPC == 0) & (s > 0))
            def _():
                chunk_wait(s // SPC)
            return step(s, m)

        m_fin = lax.fori_loop(0, NSEG - 1, step_w, m0)
    step(NSEG - 1, m_fin, last=True)

    awo_copy.wait()

    OB = CFG.get("oblocks", (512, 512, 512, 512))
    OOFF = [sum(OB[:i]) for i in range(len(OB))]

    def oa_copy(i):
        return pltpu.make_async_copy(xa.at[pl.ds(OOFF[i], OB[i]), :],
                                     out_hbm.at[pl.ds(OOFF[i], OB[i]), pl.ds(0, D)], sem_oa.at[i])

    for i in range(len(OB)):
        o_t = _upk(ot[:, OOFF[i]:OOFF[i] + OB[i]])
        r = lax.dot_general(o_t, awo[...], (((0,), (0,)), ((), ())), preferred_element_type=f32)
        xa[OOFF[i]:OOFF[i] + OB[i], :] = r.astype(bf16)
        oa_copy(i).start()
    with jax.named_scope("final_waits") if CFG.get("scopes") else contextlib.nullcontext():
        for i in range(len(OB)):
            oa_copy(i).wait()
    if CFG.get("nsteps", NSEG) == NSEG:
        pltpu.make_async_copy(xb, out_hbm.at[:, pl.ds(D, D)], sem_ob).wait()
    else:
        n = CFG["nsteps"] * SEG
        pltpu.make_async_copy(xb.at[pl.ds(0, n), :], out_hbm.at[pl.ds(0, n), pl.ds(D, D)], sem_ob).wait()


@functools.partial(jax.jit, static_argnames=("B_seg_len",))
def pallas_concat_heads__softmax_full_mha__memory_aug_recurrent_mem_tr__prompt_kernel(
    A_x: jax.Array,
    A_wqkv: jax.Array,
    A_wo: jax.Array,
    B_x: jax.Array,
    B_mem0: jax.Array,
    B_Wq: jax.Array,
    B_Wk: jax.Array,
    B_Wv: jax.Array,
    B_Wo: jax.Array,
    B_seg_len: int = SEG,
):
    assert A_x.shape == (1, S, D) and B_x.shape == (1, S, D) and B_mem0.shape == (1, M, D)
    assert B_Wq.shape == (D, HB, DHB) and B_Wo.shape == (HB, DHB, D)
    assert int(B_seg_len) == SEG

    scratch = [
        pltpu.VMEM((S, D), bf16),
        pltpu.VMEM((D, 3 * D), bf16),
        pltpu.VMEM((D, D), bf16),
        pltpu.VMEM((8, S // 2, 128), u32),
        pltpu.VMEM((8, S // 2, 128), u32),
        pltpu.VMEM((D // 2, S), u32),
        pltpu.VMEM((D // 2, S), u32),
        pltpu.VMEM((S, D), bf16),
        pltpu.VMEM((M, D), bf16),
        (pltpu.VMEM((NSTAGE, D, 128), u32) if CFG.get('eo','stride')=='stride' else pltpu.VMEM((NSTAGE, 2, D // 2, 128), u32)),
        pltpu.VMEM((3 * HB, D // 2, 128), u32),
        pltpu.VMEM((8, HB * DHB // 2, 128), u32),
        pltpu.VMEM((L, D), f32),
        pltpu.VMEM((L, HB * DHB), f32),
        pltpu.VMEM((NQ // 2, 128), u32),
        pltpu.VMEM((D, D), bf16),
        pltpu.VMEM((8, L, 128), f32),
        pltpu.SemaphoreType.DMA((NRB + 6 + 8 + 6 + NRB,)),
        pltpu.SemaphoreType.DMA((NSTAGE,)),
        pltpu.SemaphoreType.DMA((len(CFG.get('oblocks', (512, 512, 512, 512))),)),
        pltpu.SemaphoreType.DMA,
    ] + [pltpu.VMEM((KT, NQ), f32)] * (2 * NKT)

    out = pl.pallas_call(
        _kernel,
        out_shape=jax.ShapeDtypeStruct((S, 2 * D), bf16),
        in_specs=[pl.BlockSpec(memory_space=pl.ANY)] * 9,
        out_specs=pl.BlockSpec(memory_space=pl.ANY),
        scratch_shapes=scratch,
        compiler_params=pltpu.CompilerParams(vmem_limit_bytes=112 * 1024 * 1024),
    )(A_x.reshape(S, D), A_wqkv, A_wo, B_x.reshape(S, D), B_mem0.reshape(M, D), *[(w if CFG.get('eo','stride')=='stride' else w.reshape(D // 2, 2, HB, DHB)) for w in (B_Wq, B_Wk, B_Wv)],
      B_Wo.reshape(HB * DHB, D))
    return out.reshape(1, S, 2 * D)
```

```python
import functools, contextlib

import jax
import jax.numpy as jnp
import numpy as np
from jax import lax
from jax.experimental import pallas as pl
from jax.experimental.pallas import tpu as pltpu

CFG = dict(rsub=64,pm=256,rtok=1,vt2=2,tok=1,toklag=2,pstore=1,unroll=2,qk0_early=1,groups=(1,7,10,10,10,10),oblocks=(512,512,512,256,256),wka=384,d1=2,d2=1,aslots=37,p3a={31:[0],32:[1,2],33:[3,4,5],34:[6,7]},afirst_from=33)
f32 = jnp.float32
bf16 = jnp.bfloat16
u32 = jnp.uint32

LOG2E = 1.4426950408889634

S = 2048
D = 1024
HA = 32
DHA = D // HA
HB = 32
DHB = 128
M = 8
SEG = 32
L = M + SEG
NSEG = S // SEG

NQ = 512
NQB = S // NQ
KT = 128
NKT = S // KT
NCHUNK = HA * NQB
CPS = NCHUNK // NSEG
RB = 512
NRB = S // RB
NSTAGE = 20


def _pk(x):
    return pltpu.bitcast(x, u32)


def _upk(x):
    return pltpu.bitcast(x, bf16)


def _kernel(ax_hbm, wqkv_hbm, awo_hbm, bx_hbm, mem0_hbm, wq_hbm, wk_hbm, wv_hbm, wo_hbm,
            out_hbm,
            xa, wqkv, awo, k4, q4, vt, ot, xb, mem0v, stage, wp, wop, h_ref, o_ref, qm_ref, wvt, part_ref,
            sem_in, sem_stage, sem_oa, sem_ob, *s_refs):
    sb = [s_refs[0:NKT], s_refs[NKT:2 * NKT]]

    def x_copy(rb):
        return pltpu.make_async_copy(ax_hbm.at[pl.ds(rb * RB, RB), :], xa.at[pl.ds(rb * RB, RB), :],
                                     sem_in.at[rb])

    awo_copy = pltpu.make_async_copy(awo_hbm, awo, sem_in.at[NRB + 3])
    mem_copy = pltpu.make_async_copy(mem0_hbm, mem0v, sem_in.at[NRB + 5])
    wo32 = wo_hbm.bitcast(u32)

    def wo_copy(n):
        return pltpu.make_async_copy(wo32.at[:, pl.ds(n * 128, 128)], wop.at[n], sem_in.at[NRB + 6 + n])

    wb32 = [w.bitcast(u32) for w in (wq_hbm, wk_hbm, wv_hbm)]

    class _Multi:
        def __init__(self, cps):
            self.cps = cps

        def start(self):
            for c in self.cps:
                c.start()

        def wait(self):
            for c in self.cps:
                c.wait()

    def stage_copy(i):
        hp, j = divmod(i, 3)
        slot = i % NSTAGE
        if CFG.get("eo", "stride") == "stride":
            return pltpu.make_async_copy(wb32[j].at[:, hp, :], stage.at[slot], sem_stage.at[slot])
        return _Multi([pltpu.make_async_copy(wb32[j].at[:, par, hp, :], stage.at[slot, par], sem_stage.at[slot])
                       for par in range(2)])

    tokq = []

    def attach_tok(y):
        if not tokq:
            return y
        t = tokq.pop()
        while tokq:
            t = jnp.maximum(t, tokq.pop())
        yi = pltpu.bitcast(y[0:8], jnp.int32)
        y0 = pltpu.bitcast(jnp.minimum(yi, jnp.maximum(yi, t)), u32)
        return jnp.concatenate([y0, y[8:]], axis=0)

    RSUB = CFG.get("rsub", 128)

    def repack_gen(i):
        hp, j = divmod(i, 3)
        slot = i % NSTAGE
        for r in range(0, D // 2, RSUB // 2):
            n = RSUB // 2
            if CFG.get("eo", "stride") == "stride":
                e = stage[slot, pl.ds(2 * r, n, stride=2), :]
                o = stage[slot, pl.ds(2 * r + 1, n, stride=2), :]
            else:
                e = stage[slot, 0, r:r + n, :]
                o = stage[slot, 1, r:r + n, :]
            lo = (e & jnp.uint32(0xFFFF)) | (o << 16)
            hi = (e >> 16) | (o & jnp.uint32(0xFFFF0000))
            wp[j * HB + 2 * hp, r:r + n, :] = lo
            wp[j * HB + 2 * hp + 1, r:r + n, :] = hi
            if CFG.get("rtok", 0):
                t = jnp.maximum(pltpu.bitcast(lo, jnp.int32), pltpu.bitcast(hi, jnp.int32))
                t = jnp.max(t.reshape(n // 8, 8, 128), axis=0)
                tokq.append(t)
            yield

    NSLAB = 3 * HB // 2

    PM = CFG.get("pm", 512)

    def proj_nat(j, rb, dst, scale):
        for r in range(rb * RB, (rb + 1) * RB, PM):
            xs = xa[r:r + PM, :]
            for g in range(8):
                y = jnp.dot(xs, wqkv[:, j * D + g * 128: j * D + (g + 1) * 128], preferred_element_type=f32)
                if scale is not None:
                    y = y * scale
                dst[g, r // 2:(r + PM) // 2, :] = attach_tok(_pk(y.astype(bf16)))
                yield

    def proj_t(j, rb, dst):
        for r in range(rb * RB, (rb + 1) * RB, 128):
            xs = xa[r:r + 128, :]
            y = lax.dot_general(wqkv[:, j * D:(j + 1) * D], xs, (((0,), (1,)), ((), ())),
                                preferred_element_type=f32)
            dst[:, r:r + 128] = _pk(y.astype(bf16))
            yield

    TM = CFG.get("tm", 256)

    def proj_t3(rb, dst):
        if rb == 0:
            wvt[...] = wqkv[:, 2 * D:3 * D].T
        for r in range(rb * RB, (rb + 1) * RB, 128):
            xs = xa[r:r + 128, :]
            for n0 in range(0, D, TM):
                y = lax.dot_general(wvt[n0:n0 + TM, :], xs, (((1,), (1,)), ((), ())), preferred_element_type=f32)
                dst[n0 // 2:(n0 + TM) // 2, r:r + 128] = attach_tok(_pk(y.astype(bf16)))
                yield

    def proj_t2(j, rb, dst):
        for r in range(rb * RB, (rb + 1) * RB, PM):
            xs = xa[r:r + PM, :]
            for g in range(8):
                y = jnp.dot(xs, wqkv[:, j * D + g * 128: j * D + (g + 1) * 128], preferred_element_type=f32)
                yt = _pk(y.astype(bf16).T)
                dst[g * 64:(g + 1) * 64, r:r + 128] = attach_tok(yt[:, 0:128])
                if PM > 128:
                    dst[g * 64:(g + 1) * 64, r + 128:r + PM] = yt[:, 128:]
                yield

    GROUPS = CFG.get("groups", (2, 8, 8, 10, 10, 10))
    GOFF = [sum(GROUPS[:i]) for i in range(len(GROUPS) + 1)]
    assert GOFF[-1] == NSLAB and max(GROUPS[i] + GROUPS[i + 1] for i in range(len(GROUPS) - 1)) <= NSTAGE

    def slab_group_start(g):
        for i in range(GOFF[g], GOFF[g + 1]):
            stage_copy(i).start()

    def slab_group_wait(g):
        for i in range(GOFF[g], GOFF[g + 1]):
            stage_copy(i).wait()

    def slab_group_repack(g):
        for i in range(GOFF[g], GOFF[g + 1]):
            yield from repack_gen(i)

    def interleave(main, side, n_main, n_side):
        done = 0
        for i in range(n_main):
            next(main)
            while done < (i + 1) * n_side // n_main:
                next(side)
                done += 1

    NPIECE = 3 * NRB

    def wq_half(j, hf):
        return pltpu.make_async_copy(wqkv_hbm.at[pl.ds(hf * (D // 2), D // 2), pl.ds(j * D, D)],
                                     wqkv.at[pl.ds(hf * (D // 2), D // 2), pl.ds(j * D, D)],
                                     sem_in.at[NRB + 6 + 8 + j * 2 + hf])

    def wk_cols(c0, c1, si):
        return pltpu.make_async_copy(wqkv_hbm.at[:, pl.ds(D + c0, c1 - c0)], wqkv.at[:, pl.ds(D + c0, c1 - c0)],
                                     sem_in.at[si])

    WKA = CFG.get("wka", 0)

    def xb_copy(c):
        return pltpu.make_async_copy(bx_hbm.at[pl.ds(c * RB, RB), :], xb.at[pl.ds(c * RB, RB), :],
                                     sem_in.at[NRB + 6 + 8 + 6 + c])

    class _G:
        def __init__(self, g):
            self.g = g

        def start(self):
            slab_group_start(self.g)

        def wait(self):
            slab_group_wait(self.g)

    starts = {
        -1: [wq_half(1, 0), x_copy(0), wq_half(1, 1)],
        0: [x_copy(1), x_copy(2), x_copy(3), _G(0)],
        1: [_G(1)],
        2: [wq_half(0, 0), wq_half(0, 1), _G(2)],
        4: [wq_half(2, 0), wq_half(2, 1), _G(3)],
        6: [_G(4)] + [wo_copy(n) for n in range(0, 2)],
        8: [_G(5)] + [wo_copy(n) for n in range(2, 4)],
        10: [mem_copy, xb_copy(0)] + [wo_copy(n) for n in range(4, 8)],
        12: [xb_copy(c) for c in range(1, NRB)] + ([awo_copy] if CFG.get('stop') != 'pro' else []),
    }
    waits = {
        0: [wq_half(1, 0), x_copy(0), wq_half(1, 1)],
        1: [x_copy(1), x_copy(2), x_copy(3), _G(0)],
        2: [_G(1)],
        4: [wq_half(0, 0), wq_half(0, 1), _G(2)],
        6: [wq_half(2, 0), wq_half(2, 1), _G(3)],
        8: [_G(4)] + [wo_copy(n) for n in range(0, 2)],
        10: [_G(5)] + [wo_copy(n) for n in range(2, 4)],
        12: [mem_copy, xb_copy(0)] + [wo_copy(n) for n in range(4, 8)],
    }
    if WKA:
        wk_a, wk_b = wk_cols(0, WKA, NRB + 6 + 8 + 2), wk_cols(WKA, D, NRB + 6 + 8 + 3)
        starts[-1] = [wk_a, x_copy(0), wk_b]
        waits[0] = [wk_a, x_copy(0)]
    repack_at = {1: (0, 1), 2: (1, 2), 4: (2, 2), 6: (3, 2), 8: (4, 2), 10: (5, 2)}
    lane = lax.broadcasted_iota(jnp.int32, (NQ // 2, 128), 1)

    def prep_q(ci):
        hh = ci // NQB
        qb = ci % NQB
        g = hh // 4
        hl = hh % 4
        q0 = pl.multiple_of(qb * (NQ // 2), NQ // 2)
        qq = q4[g, pl.ds(q0, NQ // 2), :]
        qm_ref[...] = jnp.where((lane >= hl * DHA) & (lane < hl * DHA + DHA), qq, jnp.zeros_like(qq))

    def qk_piece(ci, kt, sbuf, mx):
        g = (ci // NQB) // 4
        kk = _upk(k4[g, kt * KT // 2:(kt + 1) * KT // 2, :])
        qm = _upk(qm_ref[...])
        st = lax.dot_general(kk, qm, (((1,), (1,)), ((), ())), preferred_element_type=f32)
        sbuf[kt][...] = st
        pm = jnp.max(st.reshape(KT // 8, 8, NQ), axis=0)
        return pm if mx is None else jnp.maximum(mx, pm)

    def sm_piece(ci, kt, sbuf, m, l, acc, tok=None):
        hh = ci // NQB
        if tok is not None and CFG.get("tok", 0):
            mi = pltpu.bitcast(m, jnp.int32)
            m = pltpu.bitcast(jnp.minimum(mi, jnp.maximum(mi, pltpu.bitcast(tok, jnp.int32))), f32)
        p = jnp.exp2(sbuf[kt][...] - m)
        ps = jnp.sum(p.reshape(KT // 8, 8, NQ), axis=0)
        l = ps if l is None else l + ps
        h0 = pl.multiple_of(hh * (DHA // 2), DHA // 2)
        vv = _upk(vt[pl.ds(h0, DHA // 2), kt * KT:(kt + 1) * KT])
        d = jnp.dot(vv, p.astype(bf16), preferred_element_type=f32)
        acc = d if acc is None else acc + d
        return l, acc

    def recip_a(x):
        if CFG.get("fastrcp", 1):
            r = pltpu.reciprocal(x, approx=True)
            return r * (2.0 - x * r)
        return pltpu.reciprocal(x, approx=False)

    def a_finish(ci, l, acc):
        hh = ci // NQB
        qb = ci % NQB
        lt = jnp.sum(l, axis=0, keepdims=True)
        o = (acc * recip_a(lt)).astype(bf16)
        h0 = pl.multiple_of(hh * (DHA // 2), DHA // 2)
        q0 = pl.multiple_of(qb * NQ, NQ)
        ot[pl.ds(h0, DHA // 2), pl.ds(q0, NQ)] = _pk(o)

    def first_scores():
        prep_q(0)
        mx = None
        for kt in range(NKT):
            mx = qk_piece(0, kt, sb[0], mx)
        return jnp.max(mx, axis=0, keepdims=True)

    for c in starts[-1]:
        c.start()
    side, side_left, pieces_left = iter(()), 0, 0
    for p in range(NPIECE + 1):
        j, rb = divmod(p, NRB)
        if CFG.get("scopes"):
            with jax.named_scope(f"wait_{p:02d}"):
                for c in waits.get(p, []):
                    c.wait()
        else:
            for c in waits.get(p, []):
                c.wait()
        for c in starts.get(p, []):
            c.start()
        if p == NPIECE:
            break
        if p == CFG.get("qk0_at", 8) and CFG.get("qk0_early"):
            pass
        if p in repack_at:
            assert side_left == 0
            g, pieces_left = repack_at[p]
            side, side_left = slab_group_repack(g), GROUPS[g] * D // RSUB
        n_side = side_left // pieces_left if pieces_left else 0
        side_left -= n_side
        pieces_left = max(pieces_left - 1, 0)
        if j == 0 and rb == 0 and WKA:
            for r in range(0, RB, PM):
                for g in range(WKA // 128):
                    y = jnp.dot(xa[r:r + PM, :], wqkv[:, D + g * 128: D + (g + 1) * 128], preferred_element_type=f32)
                    k4[g, r // 2:(r + PM) // 2, :] = _pk(y.astype(bf16))
            wk_b.wait()
            for r in range(0, RB, PM):
                for g in range(WKA // 128, 8):
                    y = jnp.dot(xa[r:r + PM, :], wqkv[:, D + g * 128: D + (g + 1) * 128], preferred_element_type=f32)
                    k4[g, r // 2:(r + PM) // 2, :] = _pk(y.astype(bf16))
            continue
        if j == 0:
            main, n_main = proj_nat(1, rb, k4, None), 8 * RB // PM
        elif j == 1:
            main, n_main = proj_nat(0, rb, q4, (DHA ** -0.5) * LOG2E), 8 * RB // PM
        elif CFG.get("vt2", 1) == 1:
            main, n_main = proj_t2(2, rb, vt), 8 * RB // PM
        elif CFG.get("vt2", 1) == 2:
            main, n_main = proj_t3(rb, vt), RB // 128 * (D // TM)
        else:
            main, n_main = proj_t(2, rb, vt), RB // 128
        interleave(main, side, n_main, n_side)
        if CFG.get("qk0_early") and p == 7:
            m0 = first_scores()
    assert side_left == 0

    def a_gen(s, m, last):
        for j in range(CPS):
            ci = s * CPS + j
            has_next = not (last and j == CPS - 1)
            cur, nxt = sb[j % 2], sb[(j + 1) % 2]
            if has_next:
                prep_q(ci + 1)
            mx = l = acc = None
            toks = []
            for kt in range(NKT):
                if has_next:
                    mx = qk_piece(ci + 1, kt, nxt, mx)
                    toks.append(mx)
                lag = CFG.get("toklag", 1)
                tok = toks[kt - lag] if (has_next and kt - lag >= 0) else None
                if tok is not None:
                    tok = tok[0:1]
                l, acc = sm_piece(ci, kt, cur, m, l, acc, tok)
                if kt == NKT - 1:
                    a_finish(ci, l, acc)
                    if has_next:
                        m = jnp.max(mx, axis=0, keepdims=True)
                yield m

    cb = (DHB ** -0.5) * LOG2E
    row = lax.broadcasted_iota(jnp.int32, (L, L), 0)
    col = lax.broadcasted_iota(jnp.int32, (L, L), 1)
    mask = (row < M) | (row >= col)
    KSPLIT = CFG.get('ksplit', 24) * DHB
    D1, D2 = CFG.get('d1', 1), CFG.get('d2', 1)

    def ob_copy(r0):
        return pltpu.make_async_copy(xb.at[pl.ds(r0, SEG), :], out_hbm.at[pl.ds(r0, SEG), pl.ds(D, D)], sem_ob)

    def recip(x):
        if CFG.get("fastrcp", 1):
            r = pltpu.reciprocal(x, approx=True)
            return r * (2.0 - x * r)
        return pltpu.reciprocal(x, approx=False)

    def step(s, m, last=False):
        r0 = s * SEG if isinstance(s, int) else pl.multiple_of(s * SEG, SEG)
        h_ref[M:L, :] = xb[pl.ds(r0, SEG), :].astype(f32)
        R0 = M if (last and CFG.get("deadrows", 1)) else 0
        ag = a_gen(s, m, last)
        npieces = CPS * NKT
        state = dict(done=0, m=m)
        st = {}
        nslots = HB + D1 + D2
        aslots = CFG.get("aslots", nslots)

        def a_upto(n):
            while state["done"] < min(npieces, n):
                state["m"] = next(ag)
                state["done"] += 1

        parts = {}
        o1 = {}

        def p3a(n):
            if "v" not in o1:
                o1["v"] = o_ref[R0:L, :KSPLIT]
            parts[n] = jnp.dot(o1["v"], _upk(wop[n, :KSPLIT // 2, :]), preferred_element_type=f32)
            if CFG.get("pstore"):
                part_ref[n, R0:L] = parts[n]
                parts[n] = None

        p3a_sched = CFG.get("p3a", {32: [0, 1, 2, 3], 33: [4, 5, 6, 7]})
        for t in range(nslots):
            if t >= CFG.get("afirst_from", 99):
                a_upto((t + 1) * npieces // aslots)
            if t < HB:
                hs = h_ref[...]
                q = jnp.dot(h_ref[R0:L, :] if R0 else hs, _upk(wp[t]), preferred_element_type=f32) * cb
                k = jnp.dot(hs, _upk(wp[HB + t]), preferred_element_type=f32)
                v = jnp.dot(hs, _upk(wp[2 * HB + t]), preferred_element_type=f32)
                st[t] = dict(q=q, k=k.astype(bf16), v=v.astype(bf16))
            hd = t - D1
            if 0 <= hd < HB:
                e = st[hd]
                sc = lax.dot_general(e["q"], e["k"], (((1,), (1,)), ((), ())), preferred_element_type=f32)
                sc = jnp.where(mask[R0:L], sc, -1e9 * LOG2E)
                mm = jnp.max(sc, axis=1, keepdims=True)
                p = jnp.exp2(sc - mm)
                e["p"] = p
                e["r"] = recip(jnp.sum(p, axis=1, keepdims=True))
            hd = t - D1 - D2
            if 0 <= hd < HB:
                e = st.pop(hd)
                o = jnp.dot(e["p"], e["v"], preferred_element_type=f32) * e["r"]
                o_ref[R0:L, hd * DHB:(hd + 1) * DHB] = o
            a_upto((t + 1) * npieces // aslots)
            for n in p3a_sched.get(t, []):
                p3a(n)
        for n in range(8):
            if n not in parts:
                p3a(n)
        o2 = o_ref[R0:L, KSPLIT:]
        for n in range(8):
            pn = parts[n] if parts[n] is not None else part_ref[n, R0:L]
            r = pn + jnp.dot(o2, _upk(wop[n, KSPLIT // 2:, :]), preferred_element_type=f32)
            ob = r.astype(bf16)
            if R0:
                xb[pl.ds(r0, SEG), n * 128:(n + 1) * 128] = ob
            else:
                xb[pl.ds(r0, SEG), n * 128:(n + 1) * 128] = ob[M:L]
                h_ref[0:M, n * 128:(n + 1) * 128] = ob[0:M].astype(f32)
        a_upto(npieces)
        ob_copy(r0).start()
        return state["m"]

    h_ref[0:M, :] = mem0v[...].astype(f32)
    if not CFG.get("qk0_early"):
        m0 = first_scores()

    if CFG.get("stop") == "pro":
        ot[0:8, 0:NQ] = pltpu.bitcast(jnp.broadcast_to(m0, (8, NQ)), u32)
        return
    SPC = RB // SEG

    def chunk_wait(c):
        c0 = pl.multiple_of(c * RB, RB)
        pltpu.make_async_copy(bx_hbm.at[pl.ds(c0, RB), :], xb.at[pl.ds(c0, RB), :],
                              sem_in.at[NRB + 6 + 8 + 6 + c]).wait()

    UN = CFG.get("unroll", 1)
    if UN == 2:
        def step2(i, m):
            @pl.when((i % (SPC // 2) == 0) & (i > 0))
            def _():
                chunk_wait(i // (SPC // 2))
            m = step(2 * i, m)
            return step(2 * i + 1, m)

        m_fin = lax.fori_loop(0, NSEG // 2 - 1, step2, m0)
        m_fin = step(NSEG - 2, m_fin)
    elif CFG.get("nested", 1):
        def outer(c, m):
            @pl.when(c > 0)
            def _():
                chunk_wait(c)
            n = jnp.where(c == NRB - 1, SPC - 1, SPC)
            return lax.fori_loop(0, n, lambda i, mm: step(c * SPC + i, mm), m)

        m_fin = lax.fori_loop(0, NRB, outer, m0)
    else:
        def step_w(s, m):
            @pl.when((s % SPC == 0) & (s > 0))
            def _():
                chunk_wait(s // SPC)
            return step(s, m)

        m_fin = lax.fori_loop(0, NSEG - 1, step_w, m0)
    step(NSEG - 1, m_fin, last=True)

    awo_copy.wait()

    OB = CFG.get("oblocks", (512, 512, 512, 512))
    OOFF = [sum(OB[:i]) for i in range(len(OB))]

    def oa_copy(i):
        return pltpu.make_async_copy(xa.at[pl.ds(OOFF[i], OB[i]), :],
                                     out_hbm.at[pl.ds(OOFF[i], OB[i]), pl.ds(0, D)], sem_oa.at[i])

    for i in range(len(OB)):
        o_t = _upk(ot[:, OOFF[i]:OOFF[i] + OB[i]])
        r = lax.dot_general(o_t, awo[...], (((0,), (0,)), ((), ())), preferred_element_type=f32)
        xa[OOFF[i]:OOFF[i] + OB[i], :] = r.astype(bf16)
        oa_copy(i).start()
    with jax.named_scope("final_waits") if CFG.get("scopes") else contextlib.nullcontext():
        for i in range(len(OB)):
            oa_copy(i).wait()
    if CFG.get("nsteps", NSEG) == NSEG:
        pltpu.make_async_copy(xb, out_hbm.at[:, pl.ds(D, D)], sem_ob).wait()
    else:
        n = CFG["nsteps"] * SEG
        pltpu.make_async_copy(xb.at[pl.ds(0, n), :], out_hbm.at[pl.ds(0, n), pl.ds(D, D)], sem_ob).wait()


@functools.partial(jax.jit, static_argnames=("B_seg_len",))
def pallas_concat_heads__softmax_full_mha__memory_aug_recurrent_mem_tr__prompt_kernel(
    A_x: jax.Array,
    A_wqkv: jax.Array,
    A_wo: jax.Array,
    B_x: jax.Array,
    B_mem0: jax.Array,
    B_Wq: jax.Array,
    B_Wk: jax.Array,
    B_Wv: jax.Array,
    B_Wo: jax.Array,
    B_seg_len: int = SEG,
):
    assert A_x.shape == (1, S, D) and B_x.shape == (1, S, D) and B_mem0.shape == (1, M, D)
    assert B_Wq.shape == (D, HB, DHB) and B_Wo.shape == (HB, DHB, D)
    assert int(B_seg_len) == SEG

    scratch = [
        pltpu.VMEM((S, D), bf16),
        pltpu.VMEM((D, 3 * D), bf16),
        pltpu.VMEM((D, D), bf16),
        pltpu.VMEM((8, S // 2, 128), u32),
        pltpu.VMEM((8, S // 2, 128), u32),
        pltpu.VMEM((D // 2, S), u32),
        pltpu.VMEM((D // 2, S), u32),
        pltpu.VMEM((S, D), bf16),
        pltpu.VMEM((M, D), bf16),
        (pltpu.VMEM((NSTAGE, D, 128), u32) if CFG.get('eo','stride')=='stride' else pltpu.VMEM((NSTAGE, 2, D // 2, 128), u32)),
        pltpu.VMEM((3 * HB, D // 2, 128), u32),
        pltpu.VMEM((8, HB * DHB // 2, 128), u32),
        pltpu.VMEM((L, D), f32),
        pltpu.VMEM((L, HB * DHB), f32),
        pltpu.VMEM((NQ // 2, 128), u32),
        pltpu.VMEM((D, D), bf16),
        pltpu.VMEM((8, L, 128), f32),
        pltpu.SemaphoreType.DMA((NRB + 6 + 8 + 6 + NRB,)),
        pltpu.SemaphoreType.DMA((NSTAGE,)),
        pltpu.SemaphoreType.DMA((len(CFG.get('oblocks', (512, 512, 512, 512))),)),
        pltpu.SemaphoreType.DMA,
    ] + [pltpu.VMEM((KT, NQ), f32)] * (2 * NKT)

    out = pl.pallas_call(
        _kernel,
        out_shape=jax.ShapeDtypeStruct((S, 2 * D), bf16),
        in_specs=[pl.BlockSpec(memory_space=pl.ANY)] * 9,
        out_specs=pl.BlockSpec(memory_space=pl.ANY),
        scratch_shapes=scratch,
        compiler_params=pltpu.CompilerParams(vmem_limit_bytes=112 * 1024 * 1024),
    )(A_x.reshape(S, D), A_wqkv, A_wo, B_x.reshape(S, D), B_mem0.reshape(M, D), *[(w if CFG.get('eo','stride')=='stride' else w.reshape(D // 2, 2, HB, DHB)) for w in (B_Wq, B_Wk, B_Wv)],
      B_Wo.reshape(HB * DHB, D))
    return out.reshape(1, S, 2 * D)
```

```python
import functools, contextlib

import jax
import jax.numpy as jnp
import numpy as np
from jax import lax
from jax.experimental import pallas as pl
from jax.experimental.pallas import tpu as pltpu

CFG = dict(rsub=64,pm=256,rtok=1,vt2=2,tok=1,pstore=1,unroll=2,qk0_early=1,groups=(1,7,10,10,10,10),oblocks=(512,512,512,256,256),wka=384,p3a={31:[0],32:[1,2],33:[3,4,5],34:[6,7]},afirst_from=33,nq=256,toklag=3,d1=2,d2=1,aslots=37)
f32 = jnp.float32
bf16 = jnp.bfloat16
u32 = jnp.uint32

LOG2E = 1.4426950408889634

S = 2048
D = 1024
HA = 32
DHA = D // HA
HB = 32
DHB = 128
M = 8
SEG = 32
L = M + SEG
NSEG = S // SEG

NQ = CFG.get("nq", 512)
NQB = S // NQ
KT = 128
NKT = S // KT
NCHUNK = HA * NQB
CPS = NCHUNK // NSEG
RB = 512
NRB = S // RB
NSTAGE = 20


def _pk(x):
    return pltpu.bitcast(x, u32)


def _upk(x):
    return pltpu.bitcast(x, bf16)


def _kernel(ax_hbm, wqkv_hbm, awo_hbm, bx_hbm, mem0_hbm, wq_hbm, wk_hbm, wv_hbm, wo_hbm,
            out_hbm,
            xa, wqkv, awo, k4, q4, vt, ot, xb, mem0v, stage, wp, wop, h_ref, o_ref, qm_ref, wvt, part_ref,
            sem_in, sem_stage, sem_oa, sem_ob, sem0, *s_refs):
    sb = [s_refs[0:NKT], s_refs[NKT:2 * NKT]]

    def x_copy(rb):
        return pltpu.make_async_copy(ax_hbm.at[pl.ds(rb * RB, RB), :], xa.at[pl.ds(rb * RB, RB), :],
                                     sem_in.at[rb])

    awo_copy = pltpu.make_async_copy(awo_hbm, awo, sem_in.at[NRB + 3])
    mem_copy = pltpu.make_async_copy(mem0_hbm, mem0v, sem_in.at[NRB + 5])
    wo32 = wo_hbm.bitcast(u32)

    def wo_copy(n):
        return pltpu.make_async_copy(wo32.at[:, pl.ds(n * 128, 128)], wop.at[n], sem_in.at[NRB + 6 + n])

    wb32 = [w.bitcast(u32) for w in (wq_hbm, wk_hbm, wv_hbm)]

    class _Multi:
        def __init__(self, cps):
            self.cps = cps

        def start(self):
            for c in self.cps:
                c.start()

        def wait(self):
            for c in self.cps:
                c.wait()

    def stage_copy(i):
        hp, j = divmod(i, 3)
        slot = i % NSTAGE
        if CFG.get("eo", "stride") == "stride":
            return pltpu.make_async_copy(wb32[j].at[:, hp, :], stage.at[slot], sem_stage.at[slot])
        return _Multi([pltpu.make_async_copy(wb32[j].at[:, par, hp, :], stage.at[slot, par], sem_stage.at[slot])
                       for par in range(2)])

    tokq = []

    def attach_tok(y):
        if not tokq:
            return y
        t = tokq.pop()
        while tokq:
            t = jnp.maximum(t, tokq.pop())
        yi = pltpu.bitcast(y[0:8], jnp.int32)
        y0 = pltpu.bitcast(jnp.minimum(yi, jnp.maximum(yi, t)), u32)
        return jnp.concatenate([y0, y[8:]], axis=0)

    RSUB = CFG.get("rsub", 128)

    def repack_gen(i):
        hp, j = divmod(i, 3)
        slot = i % NSTAGE
        for r in range(0, D // 2, RSUB // 2):
            n = RSUB // 2
            if CFG.get("eo", "stride") == "stride":
                e = stage[slot, pl.ds(2 * r, n, stride=2), :]
                o = stage[slot, pl.ds(2 * r + 1, n, stride=2), :]
            else:
                e = stage[slot, 0, r:r + n, :]
                o = stage[slot, 1, r:r + n, :]
            lo = (e & jnp.uint32(0xFFFF)) | (o << 16)
            hi = (e >> 16) | (o & jnp.uint32(0xFFFF0000))
            wp[j * HB + 2 * hp, r:r + n, :] = lo
            wp[j * HB + 2 * hp + 1, r:r + n, :] = hi
            if CFG.get("rtok", 0):
                t = jnp.maximum(pltpu.bitcast(lo, jnp.int32), pltpu.bitcast(hi, jnp.int32))
                t = jnp.max(t.reshape(n // 8, 8, 128), axis=0)
                tokq.append(t)
            yield

    NSLAB = 3 * HB // 2

    PM = CFG.get("pm", 512)

    def proj_nat(j, rb, dst, scale):
        for r in range(rb * RB, (rb + 1) * RB, PM):
            xs = xa[r:r + PM, :]
            for g in range(8):
                y = jnp.dot(xs, wqkv[:, j * D + g * 128: j * D + (g + 1) * 128], preferred_element_type=f32)
                if scale is not None:
                    y = y * scale
                dst[g, r // 2:(r + PM) // 2, :] = attach_tok(_pk(y.astype(bf16)))
                yield

    def proj_t(j, rb, dst):
        for r in range(rb * RB, (rb + 1) * RB, 128):
            xs = xa[r:r + 128, :]
            y = lax.dot_general(wqkv[:, j * D:(j + 1) * D], xs, (((0,), (1,)), ((), ())),
                                preferred_element_type=f32)
            dst[:, r:r + 128] = _pk(y.astype(bf16))
            yield

    TM = CFG.get("tm", 256)

    def proj_t3(rb, dst):
        if rb == 0:
            wvt[...] = wqkv[:, 2 * D:3 * D].T
        for r in range(rb * RB, (rb + 1) * RB, 128):
            xs = xa[r:r + 128, :]
            for n0 in range(0, D, TM):
                y = lax.dot_general(wvt[n0:n0 + TM, :], xs, (((1,), (1,)), ((), ())), preferred_element_type=f32)
                dst[n0 // 2:(n0 + TM) // 2, r:r + 128] = attach_tok(_pk(y.astype(bf16)))
                yield

    def proj_t2(j, rb, dst):
        for r in range(rb * RB, (rb + 1) * RB, PM):
            xs = xa[r:r + PM, :]
            for g in range(8):
                y = jnp.dot(xs, wqkv[:, j * D + g * 128: j * D + (g + 1) * 128], preferred_element_type=f32)
                yt = _pk(y.astype(bf16).T)
                dst[g * 64:(g + 1) * 64, r:r + 128] = attach_tok(yt[:, 0:128])
                if PM > 128:
                    dst[g * 64:(g + 1) * 64, r + 128:r + PM] = yt[:, 128:]
                yield

    GROUPS = CFG.get("groups", (2, 8, 8, 10, 10, 10))
    GOFF = [sum(GROUPS[:i]) for i in range(len(GROUPS) + 1)]
    assert GOFF[-1] == NSLAB and max(GROUPS[i] + GROUPS[i + 1] for i in range(len(GROUPS) - 1)) <= NSTAGE

    def slab_group_start(g):
        for i in range(GOFF[g], GOFF[g + 1]):
            stage_copy(i).start()

    def slab_group_wait(g):
        for i in range(GOFF[g], GOFF[g + 1]):
            stage_copy(i).wait()

    def slab_group_repack(g):
        for i in range(GOFF[g], GOFF[g + 1]):
            yield from repack_gen(i)

    def interleave(main, side, n_main, n_side):
        done = 0
        for i in range(n_main):
            next(main)
            while done < (i + 1) * n_side // n_main:
                next(side)
                done += 1

    NPIECE = 3 * NRB

    def wq_half(j, hf):
        return pltpu.make_async_copy(wqkv_hbm.at[pl.ds(hf * (D // 2), D // 2), pl.ds(j * D, D)],
                                     wqkv.at[pl.ds(hf * (D // 2), D // 2), pl.ds(j * D, D)],
                                     sem_in.at[NRB + 6 + 8 + j * 2 + hf])

    def wk_cols(c0, c1, si):
        return pltpu.make_async_copy(wqkv_hbm.at[:, pl.ds(D + c0, c1 - c0)], wqkv.at[:, pl.ds(D + c0, c1 - c0)],
                                     sem_in.at[si])

    WKA = CFG.get("wka", 0)

    def xb_copy(c):
        return pltpu.make_async_copy(bx_hbm.at[pl.ds(c * RB, RB), :], xb.at[pl.ds(c * RB, RB), :],
                                     sem_in.at[NRB + 6 + 8 + 6 + c])

    class _G:
        def __init__(self, g):
            self.g = g

        def start(self):
            slab_group_start(self.g)

        def wait(self):
            slab_group_wait(self.g)

    starts = {
        -1: [wq_half(1, 0), x_copy(0), wq_half(1, 1)],
        0: [x_copy(1), x_copy(2), x_copy(3), _G(0)],
        1: [_G(1)],
        2: [wq_half(0, 0), wq_half(0, 1), _G(2)],
        4: [wq_half(2, 0), wq_half(2, 1), _G(3)],
        6: [_G(4)] + [wo_copy(n) for n in range(0, 2)],
        8: [_G(5)] + [wo_copy(n) for n in range(2, 4)],
        10: [mem_copy, xb_copy(0)] + [wo_copy(n) for n in range(4, 8)],
        12: [xb_copy(c) for c in range(1, NRB)] + ([awo_copy] if CFG.get('stop') != 'pro' else []),
    }
    waits = {
        0: [wq_half(1, 0), x_copy(0), wq_half(1, 1)],
        1: [x_copy(1), x_copy(2), x_copy(3), _G(0)],
        2: [_G(1)],
        4: [wq_half(0, 0), wq_half(0, 1), _G(2)],
        6: [wq_half(2, 0), wq_half(2, 1), _G(3)],
        8: [_G(4)] + [wo_copy(n) for n in range(0, 2)],
        10: [_G(5)] + [wo_copy(n) for n in range(2, 4)],
        12: [mem_copy, xb_copy(0)] + [wo_copy(n) for n in range(4, 8)],
    }
    if WKA:
        wk_a, wk_b = wk_cols(0, WKA, NRB + 6 + 8 + 2), wk_cols(WKA, D, NRB + 6 + 8 + 3)
        starts[-1] = [wk_a, x_copy(0), wk_b]
        waits[0] = [wk_a, x_copy(0)]
        NS0 = CFG.get("split0", 0)
        if NS0:
            def rows_of(src, dst, r0, n, c0, cn, si):
                return pltpu.make_async_copy(src.at[pl.ds(r0, n), pl.ds(c0, cn)], dst.at[pl.ds(r0, n), pl.ds(c0, cn)],
                                             sem0.at[si])
            xs0 = [rows_of(ax_hbm, xa, i * RB // NS0, RB // NS0, 0, D, i) for i in range(NS0)]
            wa0 = [rows_of(wqkv_hbm, wqkv, i * D // NS0, D // NS0, D, WKA, NS0 + i) for i in range(NS0)]
            wb0 = [rows_of(wqkv_hbm, wqkv, i * D // NS0, D // NS0, D + WKA, D - WKA, 2 * NS0 + i) for i in range(NS0)]
            starts[-1] = [c for t in zip(wa0, xs0) for c in t] + wb0
            waits[0] = wa0 + xs0
            wk_b = _Multi(wb0)
    repack_at = {1: (0, 1), 2: (1, 2), 4: (2, 2), 6: (3, 2), 8: (4, 2), 10: (5, 2)}
    lane = lax.broadcasted_iota(jnp.int32, (NQ // 2, 128), 1)

    def prep_q(ci):
        hh = ci // NQB
        qb = ci % NQB
        g = hh // 4
        hl = hh % 4
        q0 = pl.multiple_of(qb * (NQ // 2), NQ // 2)
        qq = q4[g, pl.ds(q0, NQ // 2), :]
        qm_ref[...] = jnp.where((lane >= hl * DHA) & (lane < hl * DHA + DHA), qq, jnp.zeros_like(qq))

    def qk_piece(ci, kt, sbuf, mx):
        g = (ci // NQB) // 4
        kk = _upk(k4[g, kt * KT // 2:(kt + 1) * KT // 2, :])
        qm = _upk(qm_ref[...])
        st = lax.dot_general(kk, qm, (((1,), (1,)), ((), ())), preferred_element_type=f32)
        sbuf[kt][...] = st
        pm = jnp.max(st.reshape(KT // 8, 8, NQ), axis=0)
        return pm if mx is None else jnp.maximum(mx, pm)

    def sm_piece(ci, kt, sbuf, m, l, acc, tok=None):
        hh = ci // NQB
        if tok is not None and CFG.get("tok", 0):
            mi = pltpu.bitcast(m, jnp.int32)
            m = pltpu.bitcast(jnp.minimum(mi, jnp.maximum(mi, pltpu.bitcast(tok, jnp.int32))), f32)
        p = jnp.exp2(sbuf[kt][...] - m)
        ps = jnp.sum(p.reshape(KT // 8, 8, NQ), axis=0)
        l = ps if l is None else l + ps
        h0 = pl.multiple_of(hh * (DHA // 2), DHA // 2)
        vv = _upk(vt[pl.ds(h0, DHA // 2), kt * KT:(kt + 1) * KT])
        d = jnp.dot(vv, p.astype(bf16), preferred_element_type=f32)
        acc = d if acc is None else acc + d
        return l, acc

    def recip_a(x):
        if CFG.get("fastrcp", 1):
            r = pltpu.reciprocal(x, approx=True)
            return r * (2.0 - x * r)
        return pltpu.reciprocal(x, approx=False)

    def a_finish(ci, l, acc):
        hh = ci // NQB
        qb = ci % NQB
        lt = jnp.sum(l, axis=0, keepdims=True)
        o = (acc * recip_a(lt)).astype(bf16)
        h0 = pl.multiple_of(hh * (DHA // 2), DHA // 2)
        q0 = pl.multiple_of(qb * NQ, NQ)
        ot[pl.ds(h0, DHA // 2), pl.ds(q0, NQ)] = _pk(o)

    def first_scores():
        prep_q(0)
        mx = None
        for kt in range(NKT):
            mx = qk_piece(0, kt, sb[0], mx)
        return jnp.max(mx, axis=0, keepdims=True)

    for c in starts[-1]:
        c.start()
    side, side_left, pieces_left = iter(()), 0, 0
    for p in range(NPIECE + 1):
        j, rb = divmod(p, NRB)
        if CFG.get("scopes"):
            with jax.named_scope(f"wait_{p:02d}"):
                for c in waits.get(p, []):
                    c.wait()
        else:
            for c in waits.get(p, []):
                c.wait()
        for c in starts.get(p, []):
            c.start()
        if p == NPIECE:
            break
        if p == CFG.get("qk0_at", 8) and CFG.get("qk0_early"):
            pass
        if p in repack_at:
            assert side_left == 0
            g, pieces_left = repack_at[p]
            side, side_left = slab_group_repack(g), GROUPS[g] * D // RSUB
        n_side = side_left // pieces_left if pieces_left else 0
        side_left -= n_side
        pieces_left = max(pieces_left - 1, 0)
        if j == 0 and rb == 0 and WKA:
            for r in range(0, RB, PM):
                for g in range(WKA // 128):
                    y = jnp.dot(xa[r:r + PM, :], wqkv[:, D + g * 128: D + (g + 1) * 128], preferred_element_type=f32)
                    k4[g, r // 2:(r + PM) // 2, :] = _pk(y.astype(bf16))
            wk_b.wait()
            for r in range(0, RB, PM):
                for g in range(WKA // 128, 8):
                    y = jnp.dot(xa[r:r + PM, :], wqkv[:, D + g * 128: D + (g + 1) * 128], preferred_element_type=f32)
                    k4[g, r // 2:(r + PM) // 2, :] = _pk(y.astype(bf16))
            continue
        if j == 0:
            main, n_main = proj_nat(1, rb, k4, None), 8 * RB // PM
        elif j == 1:
            main, n_main = proj_nat(0, rb, q4, (DHA ** -0.5) * LOG2E), 8 * RB // PM
        elif CFG.get("vt2", 1) == 1:
            main, n_main = proj_t2(2, rb, vt), 8 * RB // PM
        elif CFG.get("vt2", 1) == 2:
            main, n_main = proj_t3(rb, vt), RB // 128 * (D // TM)
        else:
            main, n_main = proj_t(2, rb, vt), RB // 128
        interleave(main, side, n_main, n_side)
        if CFG.get("qk0_early") and p == 7:
            m0 = first_scores()
    assert side_left == 0

    def a_gen(s, m, last):
        for j in range(CPS):
            ci = s * CPS + j
            has_next = not (last and j == CPS - 1)
            cur, nxt = sb[j % 2], sb[(j + 1) % 2]
            if has_next:
                prep_q(ci + 1)
            mx = l = acc = None
            toks = []
            for kt in range(NKT):
                if has_next:
                    mx = qk_piece(ci + 1, kt, nxt, mx)
                    toks.append(mx)
                lag = CFG.get("toklag", 1)
                tok = toks[kt - lag] if (has_next and kt - lag >= 0) else None
                if tok is not None:
                    tok = tok[0:1]
                l, acc = sm_piece(ci, kt, cur, m, l, acc, tok)
                if kt == NKT - 1:
                    a_finish(ci, l, acc)
                    if has_next:
                        m = jnp.max(mx, axis=0, keepdims=True)
                yield m

    cb = (DHB ** -0.5) * LOG2E
    row = lax.broadcasted_iota(jnp.int32, (L, L), 0)
    col = lax.broadcasted_iota(jnp.int32, (L, L), 1)
    mask = (row < M) | (row >= col)
    KSPLIT = CFG.get('ksplit', 24) * DHB
    D1, D2 = CFG.get('d1', 1), CFG.get('d2', 1)

    def ob_copy(r0):
        return pltpu.make_async_copy(xb.at[pl.ds(r0, SEG), :], out_hbm.at[pl.ds(r0, SEG), pl.ds(D, D)], sem_ob)

    def recip(x):
        if CFG.get("fastrcp", 1):
            r = pltpu.reciprocal(x, approx=True)
            return r * (2.0 - x * r)
        return pltpu.reciprocal(x, approx=False)

    def step(s, m, last=False):
        r0 = s * SEG if isinstance(s, int) else pl.multiple_of(s * SEG, SEG)
        h_ref[M:L, :] = xb[pl.ds(r0, SEG), :].astype(f32)
        R0 = M if (last and CFG.get("deadrows", 1)) else 0
        ag = a_gen(s, m, last)
        npieces = CPS * NKT
        state = dict(done=0, m=m)
        st = {}
        nslots = HB + D1 + D2
        aslots = CFG.get("aslots", nslots)

        def a_upto(n):
            while state["done"] < min(npieces, n):
                state["m"] = next(ag)
                state["done"] += 1

        parts = {}
        o1 = {}

        def p3a(n):
            if "v" not in o1:
                o1["v"] = o_ref[R0:L, :KSPLIT]
            parts[n] = jnp.dot(o1["v"], _upk(wop[n, :KSPLIT // 2, :]), preferred_element_type=f32)
            if CFG.get("pstore"):
                part_ref[n, R0:L] = parts[n]
                parts[n] = None

        p3a_sched = CFG.get("p3a", {32: [0, 1, 2, 3], 33: [4, 5, 6, 7]})
        for t in range(nslots):
            if t >= CFG.get("afirst_from", 99):
                a_upto((t + 1) * npieces // aslots)
            if t < HB:
                hs = h_ref[...]
                q = jnp.dot(h_ref[R0:L, :] if R0 else hs, _upk(wp[t]), preferred_element_type=f32) * cb
                k = jnp.dot(hs, _upk(wp[HB + t]), preferred_element_type=f32)
                v = jnp.dot(hs, _upk(wp[2 * HB + t]), preferred_element_type=f32)
                st[t] = dict(q=q, k=k.astype(bf16), v=v.astype(bf16))
            hd = t - D1
            if 0 <= hd < HB:
                e = st[hd]
                sc = lax.dot_general(e["q"], e["k"], (((1,), (1,)), ((), ())), preferred_element_type=f32)
                sc = jnp.where(mask[R0:L], sc, -1e9 * LOG2E)
                mm = jnp.max(sc, axis=1, keepdims=True)
                p = jnp.exp2(sc - mm)
                e["p"] = p
                e["r"] = recip(jnp.sum(p, axis=1, keepdims=True))
            hd = t - D1 - D2
            if 0 <= hd < HB:
                e = st.pop(hd)
                o = jnp.dot(e["p"], e["v"], preferred_element_type=f32) * e["r"]
                o_ref[R0:L, hd * DHB:(hd + 1) * DHB] = o
            a_upto((t + 1) * npieces // aslots)
            for n in p3a_sched.get(t, []):
                p3a(n)
        for n in range(8):
            if n not in parts:
                p3a(n)
        o2 = o_ref[R0:L, KSPLIT:]
        for n in range(8):
            pn = parts[n] if parts[n] is not None else part_ref[n, R0:L]
            r = pn + jnp.dot(o2, _upk(wop[n, KSPLIT // 2:, :]), preferred_element_type=f32)
            ob = r.astype(bf16)
            if R0:
                xb[pl.ds(r0, SEG), n * 128:(n + 1) * 128] = ob
            else:
                xb[pl.ds(r0, SEG), n * 128:(n + 1) * 128] = ob[M:L]
                h_ref[0:M, n * 128:(n + 1) * 128] = ob[0:M].astype(f32)
        a_upto(npieces)
        ob_copy(r0).start()
        return state["m"]

    h_ref[0:M, :] = mem0v[...].astype(f32)
    if not CFG.get("qk0_early"):
        m0 = first_scores()

    if CFG.get("stop") == "pro":
        ot[0:8, 0:NQ] = pltpu.bitcast(jnp.broadcast_to(m0, (8, NQ)), u32)
        return
    SPC = RB // SEG

    def chunk_wait(c):
        c0 = pl.multiple_of(c * RB, RB)
        pltpu.make_async_copy(bx_hbm.at[pl.ds(c0, RB), :], xb.at[pl.ds(c0, RB), :],
                              sem_in.at[NRB + 6 + 8 + 6 + c]).wait()

    UN = CFG.get("unroll", 1)
    if UN == 2:
        def step2(i, m):
            @pl.when((i % (SPC // 2) == 0) & (i > 0))
            def _():
                chunk_wait(i // (SPC // 2))
            m = step(2 * i, m)
            return step(2 * i + 1, m)

        m_fin = lax.fori_loop(0, NSEG // 2 - 1, step2, m0)
        m_fin = step(NSEG - 2, m_fin)
    elif UN == 4:
        def step4(i, m):
            @pl.when((i % (SPC // 4) == 0) & (i > 0))
            def _():
                chunk_wait(i // (SPC // 4))
            for u in range(4):
                m = step(4 * i + u, m)
            return m

        m_fin = lax.fori_loop(0, NSEG // 4 - 1, step4, m0)
        for u in range(NSEG - 4, NSEG - 1):
            m_fin = step(u, m_fin)
    elif CFG.get("nested", 1):
        def outer(c, m):
            @pl.when(c > 0)
            def _():
                chunk_wait(c)
            n = jnp.where(c == NRB - 1, SPC - 1, SPC)
            return lax.fori_loop(0, n, lambda i, mm: step(c * SPC + i, mm), m)

        m_fin = lax.fori_loop(0, NRB, outer, m0)
    else:
        def step_w(s, m):
            @pl.when((s % SPC == 0) & (s > 0))
            def _():
                chunk_wait(s // SPC)
            return step(s, m)

        m_fin = lax.fori_loop(0, NSEG - 1, step_w, m0)
    step(NSEG - 1, m_fin, last=True)

    awo_copy.wait()

    OB = CFG.get("oblocks", (512, 512, 512, 512))
    OOFF = [sum(OB[:i]) for i in range(len(OB))]

    def oa_copy(i):
        return pltpu.make_async_copy(xa.at[pl.ds(OOFF[i], OB[i]), :],
                                     out_hbm.at[pl.ds(OOFF[i], OB[i]), pl.ds(0, D)], sem_oa.at[i])

    for i in range(len(OB)):
        o_t = _upk(ot[:, OOFF[i]:OOFF[i] + OB[i]])
        r = lax.dot_general(o_t, awo[...], (((0,), (0,)), ((), ())), preferred_element_type=f32)
        xa[OOFF[i]:OOFF[i] + OB[i], :] = r.astype(bf16)
        oa_copy(i).start()
    with jax.named_scope("final_waits") if CFG.get("scopes") else contextlib.nullcontext():
        for i in range(len(OB)):
            oa_copy(i).wait()
    if CFG.get("nsteps", NSEG) == NSEG:
        pltpu.make_async_copy(xb, out_hbm.at[:, pl.ds(D, D)], sem_ob).wait()
    else:
        n = CFG["nsteps"] * SEG
        pltpu.make_async_copy(xb.at[pl.ds(0, n), :], out_hbm.at[pl.ds(0, n), pl.ds(D, D)], sem_ob).wait()


@functools.partial(jax.jit, static_argnames=("B_seg_len",))
def pallas_concat_heads__softmax_full_mha__memory_aug_recurrent_mem_tr__prompt_kernel(
    A_x: jax.Array,
    A_wqkv: jax.Array,
    A_wo: jax.Array,
    B_x: jax.Array,
    B_mem0: jax.Array,
    B_Wq: jax.Array,
    B_Wk: jax.Array,
    B_Wv: jax.Array,
    B_Wo: jax.Array,
    B_seg_len: int = SEG,
):
    assert A_x.shape == (1, S, D) and B_x.shape == (1, S, D) and B_mem0.shape == (1, M, D)
    assert B_Wq.shape == (D, HB, DHB) and B_Wo.shape == (HB, DHB, D)
    assert int(B_seg_len) == SEG

    scratch = [
        pltpu.VMEM((S, D), bf16),
        pltpu.VMEM((D, 3 * D), bf16),
        pltpu.VMEM((D, D), bf16),
        pltpu.VMEM((8, S // 2, 128), u32),
        pltpu.VMEM((8, S // 2, 128), u32),
        pltpu.VMEM((D // 2, S), u32),
        pltpu.VMEM((D // 2, S), u32),
        pltpu.VMEM((S, D), bf16),
        pltpu.VMEM((M, D), bf16),
        (pltpu.VMEM((NSTAGE, D, 128), u32) if CFG.get('eo','stride')=='stride' else pltpu.VMEM((NSTAGE, 2, D // 2, 128), u32)),
        pltpu.VMEM((3 * HB, D // 2, 128), u32),
        pltpu.VMEM((8, HB * DHB // 2, 128), u32),
        pltpu.VMEM((L, D), f32),
        pltpu.VMEM((L, HB * DHB), f32),
        pltpu.VMEM((NQ // 2, 128), u32),
        pltpu.VMEM((D, D), bf16),
        pltpu.VMEM((8, L, 128), f32),
        pltpu.SemaphoreType.DMA((NRB + 6 + 8 + 6 + NRB,)),
        pltpu.SemaphoreType.DMA((NSTAGE,)),
        pltpu.SemaphoreType.DMA((len(CFG.get('oblocks', (512, 512, 512, 512))),)),
        pltpu.SemaphoreType.DMA,
        pltpu.SemaphoreType.DMA((24,)),
    ] + [pltpu.VMEM((KT, NQ), f32)] * (2 * NKT)

    out = pl.pallas_call(
        _kernel,
        out_shape=jax.ShapeDtypeStruct((S, 2 * D), bf16),
        in_specs=[pl.BlockSpec(memory_space=pl.ANY)] * 9,
        out_specs=pl.BlockSpec(memory_space=pl.ANY),
        scratch_shapes=scratch,
        compiler_params=pltpu.CompilerParams(vmem_limit_bytes=112 * 1024 * 1024),
    )(A_x.reshape(S, D), A_wqkv, A_wo, B_x.reshape(S, D), B_mem0.reshape(M, D), *[(w if CFG.get('eo','stride')=='stride' else w.reshape(D // 2, 2, HB, DHB)) for w in (B_Wq, B_Wk, B_Wv)],
      B_Wo.reshape(HB * DHB, D))
    return out.reshape(1, S, 2 * D)
```

```python
import functools, contextlib

import jax
import jax.numpy as jnp
import numpy as np
from jax import lax
from jax.experimental import pallas as pl
from jax.experimental.pallas import tpu as pltpu

CFG = dict(rsub=64,pm=256,rtok=1,vt2=2,tok=1,pstore=1,unroll=2,qk0_early=1,groups=(1,7,10,10,10,10),oblocks=(512,512,512,256,256),wka=384,p3a={31:[0],32:[1,2],33:[3,4,5],34:[6,7]},nq=256,toklag=3,d1=2,d2=1,aslots=37,seq='qAkvAso',seqt='sAo')
f32 = jnp.float32
bf16 = jnp.bfloat16
u32 = jnp.uint32

LOG2E = 1.4426950408889634

S = 2048
D = 1024
HA = 32
DHA = D // HA
HB = 32
DHB = 128
M = 8
SEG = 32
L = M + SEG
NSEG = S // SEG

NQ = CFG.get("nq", 512)
NQB = S // NQ
KT = 128
NKT = S // KT
NCHUNK = HA * NQB
CPS = NCHUNK // NSEG
RB = 512
NRB = S // RB
NSTAGE = 20


def _pk(x):
    return pltpu.bitcast(x, u32)


def _upk(x):
    return pltpu.bitcast(x, bf16)


def _kernel(ax_hbm, wqkv_hbm, awo_hbm, bx_hbm, mem0_hbm, wq_hbm, wk_hbm, wv_hbm, wo_hbm,
            out_hbm,
            xa, wqkv, awo, k4, q4, vt, ot, xb, mem0v, stage, wp, wop, h_ref, o_ref, qm_ref, wvt, part_ref,
            sem_in, sem_stage, sem_oa, sem_ob, sem0, *s_refs):
    sb = [s_refs[0:NKT], s_refs[NKT:2 * NKT]]

    def x_copy(rb):
        return pltpu.make_async_copy(ax_hbm.at[pl.ds(rb * RB, RB), :], xa.at[pl.ds(rb * RB, RB), :],
                                     sem_in.at[rb])

    awo_copy = pltpu.make_async_copy(awo_hbm, awo, sem_in.at[NRB + 3])
    mem_copy = pltpu.make_async_copy(mem0_hbm, mem0v, sem_in.at[NRB + 5])
    wo32 = wo_hbm.bitcast(u32)

    def wo_copy(n):
        return pltpu.make_async_copy(wo32.at[:, pl.ds(n * 128, 128)], wop.at[n], sem_in.at[NRB + 6 + n])

    wb32 = [w.bitcast(u32) for w in (wq_hbm, wk_hbm, wv_hbm)]

    class _Multi:
        def __init__(self, cps):
            self.cps = cps

        def start(self):
            for c in self.cps:
                c.start()

        def wait(self):
            for c in self.cps:
                c.wait()

    def stage_copy(i):
        hp, j = divmod(i, 3)
        slot = i % NSTAGE
        if CFG.get("eo", "stride") == "stride":
            return pltpu.make_async_copy(wb32[j].at[:, hp, :], stage.at[slot], sem_stage.at[slot])
        return _Multi([pltpu.make_async_copy(wb32[j].at[:, par, hp, :], stage.at[slot, par], sem_stage.at[slot])
                       for par in range(2)])

    tokq = []

    def attach_tok(y):
        if not tokq:
            return y
        t = tokq.pop()
        while tokq:
            t = jnp.maximum(t, tokq.pop())
        yi = pltpu.bitcast(y[0:8], jnp.int32)
        y0 = pltpu.bitcast(jnp.minimum(yi, jnp.maximum(yi, t)), u32)
        return jnp.concatenate([y0, y[8:]], axis=0)

    RSUB = CFG.get("rsub", 128)

    def repack_gen(i):
        hp, j = divmod(i, 3)
        slot = i % NSTAGE
        for r in range(0, D // 2, RSUB // 2):
            n = RSUB // 2
            if CFG.get("eo", "stride") == "stride":
                e = stage[slot, pl.ds(2 * r, n, stride=2), :]
                o = stage[slot, pl.ds(2 * r + 1, n, stride=2), :]
            else:
                e = stage[slot, 0, r:r + n, :]
                o = stage[slot, 1, r:r + n, :]
            lo = (e & jnp.uint32(0xFFFF)) | (o << 16)
            hi = (e >> 16) | (o & jnp.uint32(0xFFFF0000))
            wp[j * HB + 2 * hp, r:r + n, :] = lo
            wp[j * HB + 2 * hp + 1, r:r + n, :] = hi
            if CFG.get("rtok", 0):
                t = jnp.maximum(pltpu.bitcast(lo, jnp.int32), pltpu.bitcast(hi, jnp.int32))
                t = jnp.max(t.reshape(n // 8, 8, 128), axis=0)
                tokq.append(t)
            yield

    NSLAB = 3 * HB // 2

    PM = CFG.get("pm", 512)

    def proj_nat(j, rb, dst, scale):
        for r in range(rb * RB, (rb + 1) * RB, PM):
            xs = xa[r:r + PM, :]
            for g in range(8):
                y = jnp.dot(xs, wqkv[:, j * D + g * 128: j * D + (g + 1) * 128], preferred_element_type=f32)
                if scale is not None:
                    y = y * scale
                dst[g, r // 2:(r + PM) // 2, :] = attach_tok(_pk(y.astype(bf16)))
                yield

    def proj_t(j, rb, dst):
        for r in range(rb * RB, (rb + 1) * RB, 128):
            xs = xa[r:r + 128, :]
            y = lax.dot_general(wqkv[:, j * D:(j + 1) * D], xs, (((0,), (1,)), ((), ())),
                                preferred_element_type=f32)
            dst[:, r:r + 128] = _pk(y.astype(bf16))
            yield

    TM = CFG.get("tm", 256)

    def proj_t3(rb, dst):
        if rb == 0:
            wvt[...] = wqkv[:, 2 * D:3 * D].T
        for r in range(rb * RB, (rb + 1) * RB, 128):
            xs = xa[r:r + 128, :]
            for n0 in range(0, D, TM):
                y = lax.dot_general(wvt[n0:n0 + TM, :], xs, (((1,), (1,)), ((), ())), preferred_element_type=f32)
                dst[n0 // 2:(n0 + TM) // 2, r:r + 128] = attach_tok(_pk(y.astype(bf16)))
                yield

    def proj_t2(j, rb, dst):
        for r in range(rb * RB, (rb + 1) * RB, PM):
            xs = xa[r:r + PM, :]
            for g in range(8):
                y = jnp.dot(xs, wqkv[:, j * D + g * 128: j * D + (g + 1) * 128], preferred_element_type=f32)
                yt = _pk(y.astype(bf16).T)
                dst[g * 64:(g + 1) * 64, r:r + 128] = attach_tok(yt[:, 0:128])
                if PM > 128:
                    dst[g * 64:(g + 1) * 64, r + 128:r + PM] = yt[:, 128:]
                yield

    GROUPS = CFG.get("groups", (2, 8, 8, 10, 10, 10))
    GOFF = [sum(GROUPS[:i]) for i in range(len(GROUPS) + 1)]
    assert GOFF[-1] == NSLAB and max(GROUPS[i] + GROUPS[i + 1] for i in range(len(GROUPS) - 1)) <= NSTAGE

    def slab_group_start(g):
        for i in range(GOFF[g], GOFF[g + 1]):
            stage_copy(i).start()

    def slab_group_wait(g):
        for i in range(GOFF[g], GOFF[g + 1]):
            stage_copy(i).wait()

    def slab_group_repack(g):
        for i in range(GOFF[g], GOFF[g + 1]):
            yield from repack_gen(i)

    def interleave(main, side, n_main, n_side):
        done = 0
        for i in range(n_main):
            next(main)
            while done < (i + 1) * n_side // n_main:
                next(side)
                done += 1

    NPIECE = 3 * NRB

    def wq_half(j, hf):
        return pltpu.make_async_copy(wqkv_hbm.at[pl.ds(hf * (D // 2), D // 2), pl.ds(j * D, D)],
                                     wqkv.at[pl.ds(hf * (D // 2), D // 2), pl.ds(j * D, D)],
                                     sem_in.at[NRB + 6 + 8 + j * 2 + hf])

    def wk_cols(c0, c1, si):
        return pltpu.make_async_copy(wqkv_hbm.at[:, pl.ds(D + c0, c1 - c0)], wqkv.at[:, pl.ds(D + c0, c1 - c0)],
                                     sem_in.at[si])

    WKA = CFG.get("wka", 0)

    def xb_copy(c):
        return pltpu.make_async_copy(bx_hbm.at[pl.ds(c * RB, RB), :], xb.at[pl.ds(c * RB, RB), :],
                                     sem_in.at[NRB + 6 + 8 + 6 + c])

    class _G:
        def __init__(self, g):
            self.g = g

        def start(self):
            slab_group_start(self.g)

        def wait(self):
            slab_group_wait(self.g)

    starts = {
        -1: [wq_half(1, 0), x_copy(0), wq_half(1, 1)],
        0: [x_copy(1), x_copy(2), x_copy(3), _G(0)],
        1: [_G(1)],
        2: [wq_half(0, 0), wq_half(0, 1), _G(2)],
        4: [wq_half(2, 0), wq_half(2, 1), _G(3)],
        6: [_G(4)] + [wo_copy(n) for n in range(0, 2)],
        8: [_G(5)] + [wo_copy(n) for n in range(2, 4)],
        10: [mem_copy, xb_copy(0)] + [wo_copy(n) for n in range(4, 8)],
        12: [xb_copy(c) for c in range(1, NRB)] + ([awo_copy] if CFG.get('stop') != 'pro' else []),
    }
    waits = {
        0: [wq_half(1, 0), x_copy(0), wq_half(1, 1)],
        1: [x_copy(1), x_copy(2), x_copy(3), _G(0)],
        2: [_G(1)],
        4: [wq_half(0, 0), wq_half(0, 1), _G(2)],
        6: [wq_half(2, 0), wq_half(2, 1), _G(3)],
        8: [_G(4)] + [wo_copy(n) for n in range(0, 2)],
        10: [_G(5)] + [wo_copy(n) for n in range(2, 4)],
        12: [mem_copy, xb_copy(0)] + [wo_copy(n) for n in range(4, 8)],
    }
    if WKA:
        wk_a, wk_b = wk_cols(0, WKA, NRB + 6 + 8 + 2), wk_cols(WKA, D, NRB + 6 + 8 + 3)
        starts[-1] = [wk_a, x_copy(0), wk_b]
        waits[0] = [wk_a, x_copy(0)]
        NS0 = CFG.get("split0", 0)
        if NS0:
            def rows_of(src, dst, r0, n, c0, cn, si):
                return pltpu.make_async_copy(src.at[pl.ds(r0, n), pl.ds(c0, cn)], dst.at[pl.ds(r0, n), pl.ds(c0, cn)],
                                             sem0.at[si])
            xs0 = [rows_of(ax_hbm, xa, i * RB // NS0, RB // NS0, 0, D, i) for i in range(NS0)]
            wa0 = [rows_of(wqkv_hbm, wqkv, i * D // NS0, D // NS0, D, WKA, NS0 + i) for i in range(NS0)]
            wb0 = [rows_of(wqkv_hbm, wqkv, i * D // NS0, D // NS0, D + WKA, D - WKA, 2 * NS0 + i) for i in range(NS0)]
            starts[-1] = [c for t in zip(wa0, xs0) for c in t] + wb0
            waits[0] = wa0 + xs0
            wk_b = _Multi(wb0)
    repack_at = {1: (0, 1), 2: (1, 2), 4: (2, 2), 6: (3, 2), 8: (4, 2), 10: (5, 2)}
    lane = lax.broadcasted_iota(jnp.int32, (NQ // 2, 128), 1)

    def prep_q(ci):
        hh = ci // NQB
        qb = ci % NQB
        g = hh // 4
        hl = hh % 4
        q0 = pl.multiple_of(qb * (NQ // 2), NQ // 2)
        qq = q4[g, pl.ds(q0, NQ // 2), :]
        qm_ref[...] = jnp.where((lane >= hl * DHA) & (lane < hl * DHA + DHA), qq, jnp.zeros_like(qq))

    def qk_piece(ci, kt, sbuf, mx):
        g = (ci // NQB) // 4
        kk = _upk(k4[g, kt * KT // 2:(kt + 1) * KT // 2, :])
        qm = _upk(qm_ref[...])
        st = lax.dot_general(kk, qm, (((1,), (1,)), ((), ())), preferred_element_type=f32)
        sbuf[kt][...] = st
        pm = jnp.max(st.reshape(KT // 8, 8, NQ), axis=0)
        return pm if mx is None else jnp.maximum(mx, pm)

    def sm_piece(ci, kt, sbuf, m, l, acc, tok=None):
        hh = ci // NQB
        if tok is not None and CFG.get("tok", 0):
            mi = pltpu.bitcast(m, jnp.int32)
            m = pltpu.bitcast(jnp.minimum(mi, jnp.maximum(mi, pltpu.bitcast(tok, jnp.int32))), f32)
        p = jnp.exp2(sbuf[kt][...] - m)
        ps = jnp.sum(p.reshape(KT // 8, 8, NQ), axis=0)
        l = ps if l is None else l + ps
        h0 = pl.multiple_of(hh * (DHA // 2), DHA // 2)
        vv = _upk(vt[pl.ds(h0, DHA // 2), kt * KT:(kt + 1) * KT])
        d = jnp.dot(vv, p.astype(bf16), preferred_element_type=f32)
        acc = d if acc is None else acc + d
        return l, acc

    def recip_a(x):
        if CFG.get("fastrcp", 1):
            r = pltpu.reciprocal(x, approx=True)
            return r * (2.0 - x * r)
        return pltpu.reciprocal(x, approx=False)

    def a_finish(ci, l, acc):
        hh = ci // NQB
        qb = ci % NQB
        lt = jnp.sum(l, axis=0, keepdims=True)
        o = (acc * recip_a(lt)).astype(bf16)
        h0 = pl.multiple_of(hh * (DHA // 2), DHA // 2)
        q0 = pl.multiple_of(qb * NQ, NQ)
        ot[pl.ds(h0, DHA // 2), pl.ds(q0, NQ)] = _pk(o)

    def first_scores():
        prep_q(0)
        mx = None
        for kt in range(NKT):
            mx = qk_piece(0, kt, sb[0], mx)
        return jnp.max(mx, axis=0, keepdims=True)

    for c in starts[-1]:
        c.start()
    side, side_left, pieces_left = iter(()), 0, 0
    for p in range(NPIECE + 1):
        j, rb = divmod(p, NRB)
        if CFG.get("scopes"):
            with jax.named_scope(f"wait_{p:02d}"):
                for c in waits.get(p, []):
                    c.wait()
        else:
            for c in waits.get(p, []):
                c.wait()
        for c in starts.get(p, []):
            c.start()
        if p == NPIECE:
            break
        if p == CFG.get("qk0_at", 8) and CFG.get("qk0_early"):
            pass
        if p in repack_at:
            assert side_left == 0
            g, pieces_left = repack_at[p]
            side, side_left = slab_group_repack(g), GROUPS[g] * D // RSUB
        n_side = side_left // pieces_left if pieces_left else 0
        side_left -= n_side
        pieces_left = max(pieces_left - 1, 0)
        if j == 0 and rb == 0 and WKA:
            for r in range(0, RB, PM):
                for g in range(WKA // 128):
                    y = jnp.dot(xa[r:r + PM, :], wqkv[:, D + g * 128: D + (g + 1) * 128], preferred_element_type=f32)
                    k4[g, r // 2:(r + PM) // 2, :] = _pk(y.astype(bf16))
            wk_b.wait()
            for r in range(0, RB, PM):
                for g in range(WKA // 128, 8):
                    y = jnp.dot(xa[r:r + PM, :], wqkv[:, D + g * 128: D + (g + 1) * 128], preferred_element_type=f32)
                    k4[g, r // 2:(r + PM) // 2, :] = _pk(y.astype(bf16))
            continue
        if j == 0:
            main, n_main = proj_nat(1, rb, k4, None), 8 * RB // PM
        elif j == 1:
            main, n_main = proj_nat(0, rb, q4, (DHA ** -0.5) * LOG2E), 8 * RB // PM
        elif CFG.get("vt2", 1) == 1:
            main, n_main = proj_t2(2, rb, vt), 8 * RB // PM
        elif CFG.get("vt2", 1) == 2:
            main, n_main = proj_t3(rb, vt), RB // 128 * (D // TM)
        else:
            main, n_main = proj_t(2, rb, vt), RB // 128
        interleave(main, side, n_main, n_side)
        if CFG.get("qk0_early") and p == 7:
            m0 = first_scores()
    assert side_left == 0

    def a_gen(s, m, last):
        for j in range(CPS):
            ci = s * CPS + j
            has_next = not (last and j == CPS - 1)
            cur, nxt = sb[j % 2], sb[(j + 1) % 2]
            if has_next:
                prep_q(ci + 1)
            mx = l = acc = None
            toks = []
            for kt in range(NKT):
                if has_next:
                    mx = qk_piece(ci + 1, kt, nxt, mx)
                    toks.append(mx)
                lag = CFG.get("toklag", 1)
                tok = toks[kt - lag] if (has_next and kt - lag >= 0) else None
                if tok is not None:
                    tok = tok[0:1]
                l, acc = sm_piece(ci, kt, cur, m, l, acc, tok)
                if kt == NKT - 1:
                    a_finish(ci, l, acc)
                    if has_next:
                        m = jnp.max(mx, axis=0, keepdims=True)
                yield m

    cb = (DHB ** -0.5) * LOG2E
    row = lax.broadcasted_iota(jnp.int32, (L, L), 0)
    col = lax.broadcasted_iota(jnp.int32, (L, L), 1)
    mask = (row < M) | (row >= col)
    KSPLIT = CFG.get('ksplit', 24) * DHB
    D1, D2 = CFG.get('d1', 1), CFG.get('d2', 1)

    def ob_copy(r0):
        return pltpu.make_async_copy(xb.at[pl.ds(r0, SEG), :], out_hbm.at[pl.ds(r0, SEG), pl.ds(D, D)], sem_ob)

    def recip(x):
        if CFG.get("fastrcp", 1):
            r = pltpu.reciprocal(x, approx=True)
            return r * (2.0 - x * r)
        return pltpu.reciprocal(x, approx=False)

    def step(s, m, last=False):
        r0 = s * SEG if isinstance(s, int) else pl.multiple_of(s * SEG, SEG)
        h_ref[M:L, :] = xb[pl.ds(r0, SEG), :].astype(f32)
        R0 = M if (last and CFG.get("deadrows", 1)) else 0
        ag = a_gen(s, m, last)
        npieces = CPS * NKT
        state = dict(done=0, m=m)
        st = {}
        nslots = HB + D1 + D2
        aslots = CFG.get("aslots", nslots)

        def a_upto(n):
            while state["done"] < min(npieces, n):
                state["m"] = next(ag)
                state["done"] += 1

        parts = {}
        o1 = {}

        def p3a(n):
            if "v" not in o1:
                o1["v"] = o_ref[R0:L, :KSPLIT]
            parts[n] = jnp.dot(o1["v"], _upk(wop[n, :KSPLIT // 2, :]), preferred_element_type=f32)
            if CFG.get("pstore"):
                part_ref[n, R0:L] = parts[n]
                parts[n] = None

        p3a_sched = CFG.get("p3a", {32: [0, 1, 2, 3], 33: [4, 5, 6, 7]})
        seq_main = CFG.get("seq", "qAkvAso")
        seq_tail = CFG.get("seqt", seq_main)

        def att_scores(hd):
            e = st[hd]
            sc = lax.dot_general(e["q"], e["k"], (((1,), (1,)), ((), ())), preferred_element_type=f32)
            sc = jnp.where(mask[R0:L], sc, -1e9 * LOG2E)
            mm = jnp.max(sc, axis=1, keepdims=True)
            p = jnp.exp2(sc - mm)
            e["p"] = p
            e["r"] = recip(jnp.sum(p, axis=1, keepdims=True))

        def att_out(hd):
            e = st.pop(hd)
            o = jnp.dot(e["p"], e["v"], preferred_element_type=f32) * e["r"]
            o_ref[R0:L, hd * DHB:(hd + 1) * DHB] = o

        for t in range(nslots):
            seq = seq_main if t < HB else seq_tail
            target = (t + 1) * npieces // aslots
            base = state["done"]
            n_a = seq.count("A")
            i_a = 0
            if t < HB:
                st[t] = {}
            for ch in seq:
                if ch == "A":
                    i_a += 1
                    a_upto(base + int(round((target - base) * i_a / n_a)))
                elif ch in "qkv":
                    if t < HB:
                        hs = h_ref[R0:L, :] if (ch == "q" and R0) else h_ref[...]
                        y = jnp.dot(hs, _upk(wp["qkv".index(ch) * HB + t]), preferred_element_type=f32)
                        st[t][ch] = y * cb if ch == "q" else y.astype(bf16)
                elif ch == "s":
                    if 0 <= t - D1 < HB:
                        att_scores(t - D1)
                elif ch == "o":
                    if 0 <= t - D1 - D2 < HB:
                        att_out(t - D1 - D2)
                elif ch == "p":
                    for n in p3a_sched.get(t, []):
                        p3a(n)
            if "p" not in seq:
                for n in p3a_sched.get(t, []):
                    p3a(n)
        for n in range(8):
            if n not in parts:
                p3a(n)
        o2 = o_ref[R0:L, KSPLIT:]
        for n in range(8):
            pn = parts[n] if parts[n] is not None else part_ref[n, R0:L]
            r = pn + jnp.dot(o2, _upk(wop[n, KSPLIT // 2:, :]), preferred_element_type=f32)
            ob = r.astype(bf16)
            if R0:
                xb[pl.ds(r0, SEG), n * 128:(n + 1) * 128] = ob
            else:
                xb[pl.ds(r0, SEG), n * 128:(n + 1) * 128] = ob[M:L]
                h_ref[0:M, n * 128:(n + 1) * 128] = ob[0:M].astype(f32)
        a_upto(npieces)
        ob_copy(r0).start()
        return state["m"]

    h_ref[0:M, :] = mem0v[...].astype(f32)
    if not CFG.get("qk0_early"):
        m0 = first_scores()

    if CFG.get("stop") == "pro":
        ot[0:8, 0:NQ] = pltpu.bitcast(jnp.broadcast_to(m0, (8, NQ)), u32)
        return
    SPC = RB // SEG

    def chunk_wait(c):
        c0 = pl.multiple_of(c * RB, RB)
        pltpu.make_async_copy(bx_hbm.at[pl.ds(c0, RB), :], xb.at[pl.ds(c0, RB), :],
                              sem_in.at[NRB + 6 + 8 + 6 + c]).wait()

    UN = CFG.get("unroll", 1)
    if UN == 2:
        def step2(i, m):
            @pl.when((i % (SPC // 2) == 0) & (i > 0))
            def _():
                chunk_wait(i // (SPC // 2))
            m = step(2 * i, m)
            return step(2 * i + 1, m)

        m_fin = lax.fori_loop(0, NSEG // 2 - 1, step2, m0)
        m_fin = step(NSEG - 2, m_fin)
    elif UN == 4:
        def step4(i, m):
            @pl.when((i % (SPC // 4) == 0) & (i > 0))
            def _():
                chunk_wait(i // (SPC // 4))
            for u in range(4):
                m = step(4 * i + u, m)
            return m

        m_fin = lax.fori_loop(0, NSEG // 4 - 1, step4, m0)
        for u in range(NSEG - 4, NSEG - 1):
            m_fin = step(u, m_fin)
    elif CFG.get("nested", 1):
        def outer(c, m):
            @pl.when(c > 0)
            def _():
                chunk_wait(c)
            n = jnp.where(c == NRB - 1, SPC - 1, SPC)
            return lax.fori_loop(0, n, lambda i, mm: step(c * SPC + i, mm), m)

        m_fin = lax.fori_loop(0, NRB, outer, m0)
    else:
        def step_w(s, m):
            @pl.when((s % SPC == 0) & (s > 0))
            def _():
                chunk_wait(s // SPC)
            return step(s, m)

        m_fin = lax.fori_loop(0, NSEG - 1, step_w, m0)
    step(NSEG - 1, m_fin, last=True)

    awo_copy.wait()

    OB = CFG.get("oblocks", (512, 512, 512, 512))
    OOFF = [sum(OB[:i]) for i in range(len(OB))]

    def oa_copy(i):
        return pltpu.make_async_copy(xa.at[pl.ds(OOFF[i], OB[i]), :],
                                     out_hbm.at[pl.ds(OOFF[i], OB[i]), pl.ds(0, D)], sem_oa.at[i])

    for i in range(len(OB)):
        o_t = _upk(ot[:, OOFF[i]:OOFF[i] + OB[i]])
        r = lax.dot_general(o_t, awo[...], (((0,), (0,)), ((), ())), preferred_element_type=f32)
        xa[OOFF[i]:OOFF[i] + OB[i], :] = r.astype(bf16)
        oa_copy(i).start()
    with jax.named_scope("final_waits") if CFG.get("scopes") else contextlib.nullcontext():
        for i in range(len(OB)):
            oa_copy(i).wait()
    if CFG.get("nsteps", NSEG) == NSEG:
        pltpu.make_async_copy(xb, out_hbm.at[:, pl.ds(D, D)], sem_ob).wait()
    else:
        n = CFG["nsteps"] * SEG
        pltpu.make_async_copy(xb.at[pl.ds(0, n), :], out_hbm.at[pl.ds(0, n), pl.ds(D, D)], sem_ob).wait()


@functools.partial(jax.jit, static_argnames=("B_seg_len",))
def pallas_concat_heads__softmax_full_mha__memory_aug_recurrent_mem_tr__prompt_kernel(
    A_x: jax.Array,
    A_wqkv: jax.Array,
    A_wo: jax.Array,
    B_x: jax.Array,
    B_mem0: jax.Array,
    B_Wq: jax.Array,
    B_Wk: jax.Array,
    B_Wv: jax.Array,
    B_Wo: jax.Array,
    B_seg_len: int = SEG,
):
    assert A_x.shape == (1, S, D) and B_x.shape == (1, S, D) and B_mem0.shape == (1, M, D)
    assert B_Wq.shape == (D, HB, DHB) and B_Wo.shape == (HB, DHB, D)
    assert int(B_seg_len) == SEG

    scratch = [
        pltpu.VMEM((S, D), bf16),
        pltpu.VMEM((D, 3 * D), bf16),
        pltpu.VMEM((D, D), bf16),
        pltpu.VMEM((8, S // 2, 128), u32),
        pltpu.VMEM((8, S // 2, 128), u32),
        pltpu.VMEM((D // 2, S), u32),
        pltpu.VMEM((D // 2, S), u32),
        pltpu.VMEM((S, D), bf16),
        pltpu.VMEM((M, D), bf16),
        (pltpu.VMEM((NSTAGE, D, 128), u32) if CFG.get('eo','stride')=='stride' else pltpu.VMEM((NSTAGE, 2, D // 2, 128), u32)),
        pltpu.VMEM((3 * HB, D // 2, 128), u32),
        pltpu.VMEM((8, HB * DHB // 2, 128), u32),
        pltpu.VMEM((L, D), f32),
        pltpu.VMEM((L, HB * DHB), f32),
        pltpu.VMEM((NQ // 2, 128), u32),
        pltpu.VMEM((D, D), bf16),
        pltpu.VMEM((8, L, 128), f32),
        pltpu.SemaphoreType.DMA((NRB + 6 + 8 + 6 + NRB,)),
        pltpu.SemaphoreType.DMA((NSTAGE,)),
        pltpu.SemaphoreType.DMA((len(CFG.get('oblocks', (512, 512, 512, 512))),)),
        pltpu.SemaphoreType.DMA,
        pltpu.SemaphoreType.DMA((24,)),
    ] + [pltpu.VMEM((KT, NQ), f32)] * (2 * NKT)

    out = pl.pallas_call(
        _kernel,
        out_shape=jax.ShapeDtypeStruct((S, 2 * D), bf16),
        in_specs=[pl.BlockSpec(memory_space=pl.ANY)] * 9,
        out_specs=pl.BlockSpec(memory_space=pl.ANY),
        scratch_shapes=scratch,
        compiler_params=pltpu.CompilerParams(vmem_limit_bytes=112 * 1024 * 1024),
    )(A_x.reshape(S, D), A_wqkv, A_wo, B_x.reshape(S, D), B_mem0.reshape(M, D), *[(w if CFG.get('eo','stride')=='stride' else w.reshape(D // 2, 2, HB, DHB)) for w in (B_Wq, B_Wk, B_Wv)],
      B_Wo.reshape(HB * DHB, D))
    return out.reshape(1, S, 2 * D)
```

```python
import functools

import jax
import jax.numpy as jnp
from jax import lax
from jax.experimental import pallas as pl
from jax.experimental.pallas import tpu as pltpu

f32 = jnp.float32
bf16 = jnp.bfloat16
u32 = jnp.uint32
i32 = jnp.int32

LOG2E = 1.4426950408889634

S = 2048
D = 1024
HA = 32
DHA = D // HA
HB = 32
DHB = 128
M = 8
SEG = 32
L = M + SEG
NSEG = S // SEG

NQ = 256
NQB = S // NQ
KT = 128
NKT = S // KT
CPS = HA * NQB // NSEG
TIE_LAG = 3

RB = 512
NRB = S // RB
PM = 256
TM = 128
WKA = 384
NSLAB = 3 * HB // 2
GROUPS = (1, 7, 10, 10, 10, 10)
NSTAGE = 20
RSUB = 64

D1, D2 = 2, 1
NSLOT = HB + D1 + D2
ASLOTS = 37
KSPLIT = 24 * DHB
P3A_AT = {31: (0,), 32: (1, 2), 33: (3, 4, 5), 34: (6, 7)}
OBLOCKS = (512, 512, 512, 256, 256)


def _pk(x):
    return pltpu.bitcast(x, u32)


def _upk(x):
    return pltpu.bitcast(x, bf16)


def _tie(x_i32, tok_i32):
    return jnp.minimum(x_i32, jnp.maximum(x_i32, tok_i32))


def _recip(x):
    r = pltpu.reciprocal(x, approx=True)
    return r * (2.0 - x * r)


def _kernel(ax_hbm, wqkv_hbm, awo_hbm, bx_hbm, mem0_hbm, wq_hbm, wk_hbm, wv_hbm, wo_hbm,
            out_hbm,
            xa, wqkv, awo, wvt, k4, q4, vt, ot, qm_ref,
            xb, mem0v, stage, wp, wop, h_ref, o_ref, part_ref,
            sem_xa, sem_w, sem_wo, sem_xb, sem_misc, sem_stage, sem_oa, sem_ob, *s_refs):
    sbuf = (s_refs[:NKT], s_refs[NKT:])

    def rows(ref, i):
        return ref.at[pl.ds(i * RB, RB), :]

    def xa_copy(i):
        return pltpu.make_async_copy(rows(ax_hbm, i), rows(xa, i), sem_xa.at[i])

    def xb_copy(i):
        return pltpu.make_async_copy(rows(bx_hbm, i), rows(xb, i), sem_xb.at[i])

    def w_copy(r0, nr, c0, nc, si):
        return pltpu.make_async_copy(wqkv_hbm.at[pl.ds(r0, nr), pl.ds(c0, nc)],
                                     wqkv.at[pl.ds(r0, nr), pl.ds(c0, nc)], sem_w.at[si])

    wk_a = w_copy(0, D, D, WKA, 0)
    wk_b = w_copy(0, D, D + WKA, D - WKA, 1)
    wq_halves = [w_copy(h * D // 2, D // 2, 0, D, 2 + h) for h in range(2)]
    wv_halves = [w_copy(h * D // 2, D // 2, 2 * D, D, 4 + h) for h in range(2)]
    awo_copy = pltpu.make_async_copy(awo_hbm, awo, sem_misc.at[0])
    mem_copy = pltpu.make_async_copy(mem0_hbm, mem0v, sem_misc.at[1])

    wo32 = wo_hbm.bitcast(u32)

    def wo_copy(n):
        return pltpu.make_async_copy(wo32.at[:, pl.ds(n * 128, 128)], wop.at[n], sem_wo.at[n])

    wb32 = [w.bitcast(u32) for w in (wq_hbm, wk_hbm, wv_hbm)]

    def slab_copy(i):
        hp, j = divmod(i, 3)
        slot = i % NSTAGE
        return pltpu.make_async_copy(wb32[j].at[:, hp, :], stage.at[slot], sem_stage.at[slot])

    goff = [sum(GROUPS[:g]) for g in range(len(GROUPS) + 1)]

    def group(g):
        return [slab_copy(i) for i in range(goff[g], goff[g + 1])]

    def ob_copy(r0):
        return pltpu.make_async_copy(xb.at[pl.ds(r0, SEG), :], out_hbm.at[pl.ds(r0, SEG), pl.ds(D, D)], sem_ob)

    pending = []

    def tie_pending(y):
        if not pending:
            return y
        t = pending.pop()
        while pending:
            t = jnp.maximum(t, pending.pop())
        y0 = pltpu.bitcast(_tie(pltpu.bitcast(y[0:8], i32), t), u32)
        return jnp.concatenate([y0, y[8:]], axis=0)

    def retile(g):
        n = RSUB // 2
        for i in range(goff[g], goff[g + 1]):
            hp, j = divmod(i, 3)
            slot = i % NSTAGE
            for r in range(0, D // 2, n):
                ev = stage[slot, pl.ds(2 * r, n, stride=2), :]
                od = stage[slot, pl.ds(2 * r + 1, n, stride=2), :]
                lo = (ev & jnp.uint32(0xFFFF)) | (od << 16)
                hi = (ev >> 16) | (od & jnp.uint32(0xFFFF0000))
                wp[j * HB + 2 * hp, r:r + n, :] = lo
                wp[j * HB + 2 * hp + 1, r:r + n, :] = hi
                t = jnp.maximum(pltpu.bitcast(lo, i32), pltpu.bitcast(hi, i32))
                pending.append(jnp.max(t.reshape(n // 8, 8, 128), axis=0))
                yield

    def proj_dot(xs, r, j, g, dst, scale):
        y = jnp.dot(xs, wqkv[:, j * D + g * 128: j * D + (g + 1) * 128], preferred_element_type=f32)
        if scale is not None:
            y = y * scale
        dst[g, r // 2:(r + PM) // 2, :] = tie_pending(_pk(y.astype(bf16)))

    def proj_rows(rb, j, dst, scale):
        for r in range(rb * RB, (rb + 1) * RB, PM):
            xs = xa[r:r + PM, :]
            for g in range(8):
                proj_dot(xs, r, j, g, dst, scale)
                yield

    def proj_vt(rb):
        if rb == 0:
            wvt[...] = wqkv[:, 2 * D:3 * D].T
        for r in range(rb * RB, (rb + 1) * RB, 128):
            xs = xa[r:r + 128, :]
            for n0 in range(0, D, TM):
                y = lax.dot_general(wvt[n0:n0 + TM, :], xs, (((1,), (1,)), ((), ())), preferred_element_type=f32)
                vt[n0 // 2:(n0 + TM) // 2, r:r + 128] = tie_pending(_pk(y.astype(bf16)))
                yield

    lane = lax.broadcasted_iota(i32, (NQ // 2, 128), 1)

    def prep_q(ci):
        hh, qb = ci // NQB, ci % NQB
        hl = hh % 4
        qq = q4[hh // 4, pl.ds(pl.multiple_of(qb * (NQ // 2), NQ // 2), NQ // 2), :]
        qm_ref[...] = jnp.where((lane >= hl * DHA) & (lane < hl * DHA + DHA), qq, jnp.zeros_like(qq))

    def qk_piece(ci, kt, dst, mx):
        kk = _upk(k4[(ci // NQB) // 4, kt * KT // 2:(kt + 1) * KT // 2, :])
        st = lax.dot_general(kk, _upk(qm_ref[...]), (((1,), (1,)), ((), ())), preferred_element_type=f32)
        dst[kt][...] = st
        pm = jnp.max(st.reshape(KT // 8, 8, NQ), axis=0)
        return pm if mx is None else jnp.maximum(mx, pm)

    def sm_piece(ci, kt, src, m, l, acc, tok):
        if tok is not None:
            m = pltpu.bitcast(_tie(pltpu.bitcast(m, i32), pltpu.bitcast(tok, i32)), f32)
        p = jnp.exp2(src[kt][...] - m)
        ps = jnp.sum(p.reshape(KT // 8, 8, NQ), axis=0)
        h0 = pl.multiple_of((ci // NQB) * (DHA // 2), DHA // 2)
        vv = _upk(vt[pl.ds(h0, DHA // 2), kt * KT:(kt + 1) * KT])
        d = jnp.dot(vv, p.astype(bf16), preferred_element_type=f32)
        return (ps if l is None else l + ps), (d if acc is None else acc + d)

    def a_finish(ci, l, acc):
        o = (acc * _recip(jnp.sum(l, axis=0, keepdims=True))).astype(bf16)
        h0 = pl.multiple_of((ci // NQB) * (DHA // 2), DHA // 2)
        q0 = pl.multiple_of((ci % NQB) * NQ, NQ)
        ot[pl.ds(h0, DHA // 2), pl.ds(q0, NQ)] = _pk(o)

    def a_pieces(s, m, last):
        for j in range(CPS):
            ci = s * CPS + j
            has_next = not (last and j == CPS - 1)
            cur, nxt = sbuf[j % 2], sbuf[(j + 1) % 2]
            if has_next:
                prep_q(ci + 1)
            mx = l = acc = None
            toks = []
            for kt in range(NKT):
                if has_next:
                    mx = qk_piece(ci + 1, kt, nxt, mx)
                    toks.append(mx)
                tok = toks[kt - TIE_LAG][0:1] if (has_next and kt >= TIE_LAG) else None
                l, acc = sm_piece(ci, kt, cur, m, l, acc, tok)
                if kt == NKT - 1:
                    a_finish(ci, l, acc)
                    if has_next:
                        m = jnp.max(mx, axis=0, keepdims=True)
                yield m

    starts = {
        0: [xa_copy(1), xa_copy(2), xa_copy(3)] + group(0),
        1: group(1),
        2: wq_halves + group(2),
        4: wv_halves + group(3),
        6: group(4) + [wo_copy(n) for n in range(0, 2)],
        8: group(5) + [wo_copy(n) for n in range(2, 4)],
        10: [mem_copy, xb_copy(0)] + [wo_copy(n) for n in range(4, 8)],
        12: [xb_copy(c) for c in range(1, NRB)] + [awo_copy],
    }
    fences = sorted(starts)
    waits = {b: starts[a] for a, b in zip(fences[:-1], fences[1:])}
    retile_at = {1: (0, 1), 2: (1, 2), 4: (2, 2), 6: (3, 2), 8: (4, 2), 10: (5, 2)}

    for c in (wk_a, xa_copy(0), wk_b):
        c.start()
    wk_a.wait()
    xa_copy(0).wait()
    side, side_left, pieces_left = iter(()), 0, 0
    for p in range(3 * NRB + 1):
        for c in waits.get(p, ()):
            c.wait()
        for c in starts.get(p, ()):
            c.start()
        if p == 3 * NRB:
            break
        if p == 0:
            for r in range(0, RB, PM):
                for g in range(WKA // 128):
                    proj_dot(xa[r:r + PM, :], r, 1, g, k4, None)
            wk_b.wait()
            for r in range(0, RB, PM):
                for g in range(WKA // 128, 8):
                    proj_dot(xa[r:r + PM, :], r, 1, g, k4, None)
            continue
        if p in retile_at:
            g, pieces_left = retile_at[p]
            side, side_left = retile(g), GROUPS[g] * D // RSUB
        n_side = side_left // pieces_left if pieces_left else 0
        side_left -= n_side
        pieces_left = max(pieces_left - 1, 0)
        j, rb = divmod(p, NRB)
        if j == 0:
            main, n_main = proj_rows(rb, 1, k4, None), 8 * RB // PM
        elif j == 1:
            main, n_main = proj_rows(rb, 0, q4, (DHA ** -0.5) * LOG2E), 8 * RB // PM
        else:
            main, n_main = proj_vt(rb), (RB // 128) * (D // TM)
        done = 0
        for i in range(n_main):
            next(main)
            while done < (i + 1) * n_side // n_main:
                next(side)
                done += 1
        if p == 2 * NRB - 1:
            prep_q(0)
            mx = None
            for kt in range(NKT):
                mx = qk_piece(0, kt, sbuf[0], mx)
            m0 = jnp.max(mx, axis=0, keepdims=True)
    assert side_left == 0
    pending.clear()

    row = lax.broadcasted_iota(i32, (L, L), 0)
    col = lax.broadcasted_iota(i32, (L, L), 1)
    mask = (row < M) | (row >= col)
    cb = (DHB ** -0.5) * LOG2E

    def step(s, m, last=False):
        r0 = s * SEG if isinstance(s, int) else pl.multiple_of(s * SEG, SEG)
        h_ref[M:L, :] = xb[pl.ds(r0, SEG), :].astype(f32)
        q0 = M if last else 0
        gen = a_pieces(s, m, last)
        npieces = CPS * NKT
        state = dict(done=0, m=m)
        heads = {}
        o_early = []

        def a_upto(n):
            while state["done"] < min(npieces, n):
                state["m"] = next(gen)
                state["done"] += 1

        def p1(t, j):
            hs = h_ref[q0:L, :] if j == 0 else h_ref[...]
            return jnp.dot(hs, _upk(wp[j * HB + t]), preferred_element_type=f32)

        def scores(t):
            e = heads[t]
            sc = lax.dot_general(e["q"], e["k"], (((1,), (1,)), ((), ())), preferred_element_type=f32)
            sc = jnp.where(mask[q0:L], sc, -1e9 * LOG2E)
            p = jnp.exp2(sc - jnp.max(sc, axis=1, keepdims=True))
            e["p"] = p
            e["r"] = _recip(jnp.sum(p, axis=1, keepdims=True))

        def attend(t):
            e = heads.pop(t)
            o_ref[q0:L, t * DHB:(t + 1) * DHB] = jnp.dot(e["p"], e["v"], preferred_element_type=f32) * e["r"]

        def p3_early(n):
            if not o_early:
                o_early.append(o_ref[q0:L, :KSPLIT])
            part_ref[n, q0:L] = jnp.dot(o_early[0], _upk(wop[n, :KSPLIT // 2, :]), preferred_element_type=f32)

        for t in range(NSLOT):
            base = state["done"]
            target = (t + 1) * npieces // ASLOTS
            if t < HB:
                e = heads[t] = {}
                e["q"] = p1(t, 0) * cb
                a_upto(base + int(round((target - base) / 2)))
                e["k"] = p1(t, 1).astype(bf16)
                e["v"] = p1(t, 2).astype(bf16)
                a_upto(target)
            if 0 <= t - D1 < HB:
                scores(t - D1)
            if t >= HB:
                a_upto(target)
            if 0 <= t - D1 - D2 < HB:
                attend(t - D1 - D2)
            for n in P3A_AT.get(t, ()):
                p3_early(n)
        o_late = o_ref[q0:L, KSPLIT:]
        for n in range(8):
            r = part_ref[n, q0:L] + jnp.dot(o_late, _upk(wop[n, KSPLIT // 2:, :]), preferred_element_type=f32)
            ob = r.astype(bf16)
            if last:
                xb[pl.ds(r0, SEG), n * 128:(n + 1) * 128] = ob
            else:
                xb[pl.ds(r0, SEG), n * 128:(n + 1) * 128] = ob[M:L]
                h_ref[0:M, n * 128:(n + 1) * 128] = ob[0:M].astype(f32)
        a_upto(npieces)
        if not last:
            ob_copy(r0).start()
        return state["m"]

    h_ref[0:M, :] = mem0v[...].astype(f32)
    spc = RB // SEG

    def two_steps(i, m):
        @pl.when((i % (spc // 2) == 0) & (i > 0))
        def _():
            c = i // (spc // 2)
            c0 = pl.multiple_of(c * RB, RB)
            pltpu.make_async_copy(bx_hbm.at[pl.ds(c0, RB), :], xb.at[pl.ds(c0, RB), :], sem_xb.at[c]).wait()
        return step(2 * i + 1, step(2 * i, m))

    m_fin = lax.fori_loop(0, NSEG // 2 - 1, two_steps, m0)
    m_fin = step(NSEG - 2, m_fin)
    awo_copy.wait()
    step(NSEG - 1, m_fin, last=True)

    ooff = [sum(OBLOCKS[:i]) for i in range(len(OBLOCKS))]

    def oa_copy(i):
        return pltpu.make_async_copy(xa.at[pl.ds(ooff[i], OBLOCKS[i]), :],
                                     out_hbm.at[pl.ds(ooff[i], OBLOCKS[i]), pl.ds(0, D)], sem_oa.at[i])

    for i, (r0, nr) in enumerate(zip(ooff, OBLOCKS)):
        o_t = _upk(ot[:, r0:r0 + nr])
        y = lax.dot_general(o_t, awo[...], (((0,), (0,)), ((), ())), preferred_element_type=f32)
        xa[r0:r0 + nr, :] = y.astype(bf16)
        oa_copy(i).start()
        if i == 0:
            ob_copy((NSEG - 1) * SEG).start()
    for i in range(len(OBLOCKS)):
        oa_copy(i).wait()
    pltpu.make_async_copy(xb, out_hbm.at[:, pl.ds(D, D)], sem_ob).wait()


@functools.partial(jax.jit, static_argnames=("B_seg_len",))
def pallas_concat_heads__softmax_full_mha__memory_aug_recurrent_mem_tr__prompt_kernel(
    A_x: jax.Array,
    A_wqkv: jax.Array,
    A_wo: jax.Array,
    B_x: jax.Array,
    B_mem0: jax.Array,
    B_Wq: jax.Array,
    B_Wk: jax.Array,
    B_Wv: jax.Array,
    B_Wo: jax.Array,
    B_seg_len: int = SEG,
):
    assert A_x.shape == (1, S, D) and B_x.shape == (1, S, D) and B_mem0.shape == (1, M, D)
    assert A_wqkv.shape == (D, 3 * D) and A_wo.shape == (D, D)
    assert B_Wq.shape == B_Wk.shape == B_Wv.shape == (D, HB, DHB) and B_Wo.shape == (HB, DHB, D)
    assert int(B_seg_len) == SEG

    dma_sems = lambda n: pltpu.SemaphoreType.DMA((n,))
    scratch = [
        pltpu.VMEM((S, D), bf16),
        pltpu.VMEM((D, 3 * D), bf16),
        pltpu.VMEM((D, D), bf16),
        pltpu.VMEM((D, D), bf16),
        pltpu.VMEM((8, S // 2, 128), u32),
        pltpu.VMEM((8, S // 2, 128), u32),
        pltpu.VMEM((D // 2, S), u32),
        pltpu.VMEM((D // 2, S), u32),
        pltpu.VMEM((NQ // 2, 128), u32),
        pltpu.VMEM((S, D), bf16),
        pltpu.VMEM((M, D), bf16),
        pltpu.VMEM((NSTAGE, D, 128), u32),
        pltpu.VMEM((3 * HB, D // 2, 128), u32),
        pltpu.VMEM((8, HB * DHB // 2, 128), u32),
        pltpu.VMEM((L, D), f32),
        pltpu.VMEM((L, HB * DHB), f32),
        pltpu.VMEM((8, L, 128), f32),
        dma_sems(NRB), dma_sems(6), dma_sems(8), dma_sems(NRB), dma_sems(2), dma_sems(NSTAGE),
        dma_sems(len(OBLOCKS)), pltpu.SemaphoreType.DMA,
    ] + [pltpu.VMEM((KT, NQ), f32)] * (2 * NKT)

    out = pl.pallas_call(
        _kernel,
        out_shape=jax.ShapeDtypeStruct((S, 2 * D), bf16),
        in_specs=[pl.BlockSpec(memory_space=pl.ANY)] * 9,
        out_specs=pl.BlockSpec(memory_space=pl.ANY),
        scratch_shapes=scratch,
        compiler_params=pltpu.CompilerParams(vmem_limit_bytes=112 * 1024 * 1024),
    )(A_x.reshape(S, D), A_wqkv, A_wo, B_x.reshape(S, D), B_mem0.reshape(M, D), B_Wq, B_Wk, B_Wv,
      B_Wo.reshape(HB * DHB, D))
    return out.reshape(1, S, 2 * D)
```

```python
import functools

import jax
import jax.numpy as jnp
from jax import lax
from jax.experimental import pallas as pl
from jax.experimental.pallas import tpu as pltpu

f32 = jnp.float32
bf16 = jnp.bfloat16
u32 = jnp.uint32
i32 = jnp.int32

LOG2E = 1.4426950408889634

S = 2048
D = 1024
HA = 32
DHA = D // HA
HB = 32
DHB = 128
M = 8
SEG = 32
L = M + SEG
NSEG = S // SEG

NQ = 256
NQB = S // NQ
KT = 128
NKT = S // KT
CPS = HA * NQB // NSEG
TIE_LAG = 3

RB = 512
NRB = S // RB
PM = 256
TM = 128
WKA = 384
NSLAB = 3 * HB // 2
GROUPS = (3, 10, 11, 12, 12)
NSTAGE = 24
RSUB = 64

D1, D2 = 2, 1
NSLOT = HB + D1 + D2
ASLOTS = 37
KSPLIT = 24 * DHB
P3A_AT = {31: (0,), 32: (1, 2), 33: (3, 4, 5), 34: (6, 7)}
OBLOCKS = (512, 512, 512, 256, 256)


def _pk(x):
    return pltpu.bitcast(x, u32)


def _upk(x):
    return pltpu.bitcast(x, bf16)


def _tie(x_i32, tok_i32):
    return jnp.minimum(x_i32, jnp.maximum(x_i32, tok_i32))


def _recip(x):
    r = pltpu.reciprocal(x, approx=True)
    return r * (2.0 - x * r)


def _kernel(ax_hbm, wqkv_hbm, awo_hbm, bx_hbm, mem0_hbm, wq_hbm, wk_hbm, wv_hbm, wo_hbm,
            out_hbm,
            xa, wqkv, awo, wvt, k4, q4, vt, ot, qm_ref,
            xb, mem0v, stage, wp, wop, h_ref, o_ref, part_ref,
            sem_xa, sem_w, sem_wo, sem_xb, sem_misc, sem_stage, sem_oa, sem_ob, *s_refs):
    sbuf = (s_refs[:NKT], s_refs[NKT:])

    def rows(ref, i):
        return ref.at[pl.ds(i * RB, RB), :]

    def xa_copy(i):
        return pltpu.make_async_copy(rows(ax_hbm, i), rows(xa, i), sem_xa.at[i])

    def xb_copy(i):
        return pltpu.make_async_copy(rows(bx_hbm, i), rows(xb, i), sem_xb.at[i])

    X0 = 2 * SEG
    xb_head = pltpu.make_async_copy(bx_hbm.at[pl.ds(0, X0), :], xb.at[pl.ds(0, X0), :], sem_misc.at[2])
    xb_rest = pltpu.make_async_copy(bx_hbm.at[pl.ds(X0, RB - X0), :], xb.at[pl.ds(X0, RB - X0), :], sem_xb.at[0])

    def w_copy(r0, nr, c0, nc, si):
        return pltpu.make_async_copy(wqkv_hbm.at[pl.ds(r0, nr), pl.ds(c0, nc)],
                                     wqkv.at[pl.ds(r0, nr), pl.ds(c0, nc)], sem_w.at[si])

    wk_a = w_copy(0, D, D, WKA, 0)
    wk_b = w_copy(0, D, D + WKA, D - WKA, 1)
    wq_halves = [w_copy(h * D // 2, D // 2, 0, D, 2 + h) for h in range(2)]
    wv_halves = [w_copy(h * D // 2, D // 2, 2 * D, D, 4 + h) for h in range(2)]
    awo_copy = pltpu.make_async_copy(awo_hbm, awo, sem_misc.at[0])
    mem_copy = pltpu.make_async_copy(mem0_hbm, mem0v, sem_misc.at[1])

    wo32 = wo_hbm.bitcast(u32)

    def wo_copy(n):
        return pltpu.make_async_copy(wo32.at[:, pl.ds(n * 128, 128)], wop.at[n], sem_wo.at[n])

    wb32 = [w.bitcast(u32) for w in (wq_hbm, wk_hbm, wv_hbm)]

    def slab_copy(i):
        hp, j = divmod(i, 3)
        slot = i % NSTAGE
        return pltpu.make_async_copy(wb32[j].at[:, hp, :], stage.at[slot], sem_stage.at[slot])

    goff = [sum(GROUPS[:g]) for g in range(len(GROUPS) + 1)]

    def group(g):
        return [slab_copy(i) for i in range(goff[g], goff[g + 1])]

    def ob_copy(r0):
        return pltpu.make_async_copy(xb.at[pl.ds(r0, SEG), :], out_hbm.at[pl.ds(r0, SEG), pl.ds(D, D)], sem_ob)

    pending = []

    def tie_pending(y):
        if not pending:
            return y
        t = pending.pop()
        while pending:
            t = jnp.maximum(t, pending.pop())
        y0 = pltpu.bitcast(_tie(pltpu.bitcast(y[0:8], i32), t), u32)
        return jnp.concatenate([y0, y[8:]], axis=0)

    def retile(g):
        n = RSUB // 2
        for i in range(goff[g], goff[g + 1]):
            hp, j = divmod(i, 3)
            slot = i % NSTAGE
            for r in range(0, D // 2, n):
                ev = stage[slot, pl.ds(2 * r, n, stride=2), :]
                od = stage[slot, pl.ds(2 * r + 1, n, stride=2), :]
                lo = (ev & jnp.uint32(0xFFFF)) | (od << 16)
                hi = (ev >> 16) | (od & jnp.uint32(0xFFFF0000))
                wp[j * HB + 2 * hp, r:r + n, :] = lo
                wp[j * HB + 2 * hp + 1, r:r + n, :] = hi
                t = jnp.maximum(pltpu.bitcast(lo, i32), pltpu.bitcast(hi, i32))
                pending.append(jnp.max(t.reshape(n // 8, 8, 128), axis=0))
                yield

    def proj_dot(xs, r, j, g, dst, scale):
        y = jnp.dot(xs, wqkv[:, j * D + g * 128: j * D + (g + 1) * 128], preferred_element_type=f32)
        if scale is not None:
            y = y * scale
        dst[g, r // 2:(r + PM) // 2, :] = tie_pending(_pk(y.astype(bf16)))

    def proj_rows(rb, j, dst, scale):
        for r in range(rb * RB, (rb + 1) * RB, PM):
            xs = xa[r:r + PM, :]
            for g in range(8):
                proj_dot(xs, r, j, g, dst, scale)
                yield

    def proj_vt(rb):
        if rb == 0:
            wvt[...] = wqkv[:, 2 * D:3 * D].T
        for r in range(rb * RB, (rb + 1) * RB, 128):
            xs = xa[r:r + 128, :]
            for n0 in range(0, D, TM):
                y = lax.dot_general(wvt[n0:n0 + TM, :], xs, (((1,), (1,)), ((), ())), preferred_element_type=f32)
                vt[n0 // 2:(n0 + TM) // 2, r:r + 128] = tie_pending(_pk(y.astype(bf16)))
                yield

    lane = lax.broadcasted_iota(i32, (NQ // 2, 128), 1)

    def prep_q(ci):
        hh, qb = ci // NQB, ci % NQB
        hl = hh % 4
        qq = q4[hh // 4, pl.ds(pl.multiple_of(qb * (NQ // 2), NQ // 2), NQ // 2), :]
        qm_ref[...] = jnp.where((lane >= hl * DHA) & (lane < hl * DHA + DHA), qq, jnp.zeros_like(qq))

    def qk_piece(ci, kt, dst, mx):
        kk = _upk(k4[(ci // NQB) // 4, kt * KT // 2:(kt + 1) * KT // 2, :])
        st = lax.dot_general(kk, _upk(qm_ref[...]), (((1,), (1,)), ((), ())), preferred_element_type=f32)
        dst[kt][...] = st
        pm = jnp.max(st.reshape(KT // 8, 8, NQ), axis=0)
        return pm if mx is None else jnp.maximum(mx, pm)

    def sm_piece(ci, kt, src, m, l, acc, tok):
        if tok is not None:
            m = pltpu.bitcast(_tie(pltpu.bitcast(m, i32), pltpu.bitcast(tok, i32)), f32)
        p = jnp.exp2(src[kt][...] - m)
        ps = jnp.sum(p.reshape(KT // 8, 8, NQ), axis=0)
        h0 = pl.multiple_of((ci // NQB) * (DHA // 2), DHA // 2)
        vv = _upk(vt[pl.ds(h0, DHA // 2), kt * KT:(kt + 1) * KT])
        d = jnp.dot(vv, p.astype(bf16), preferred_element_type=f32)
        return (ps if l is None else l + ps), (d if acc is None else acc + d)

    def a_finish(ci, l, acc):
        o = (acc * _recip(jnp.sum(l, axis=0, keepdims=True))).astype(bf16)
        h0 = pl.multiple_of((ci // NQB) * (DHA // 2), DHA // 2)
        q0 = pl.multiple_of((ci % NQB) * NQ, NQ)
        ot[pl.ds(h0, DHA // 2), pl.ds(q0, NQ)] = _pk(o)

    def a_pieces(s, m, last):
        for j in range(CPS):
            ci = s * CPS + j
            has_next = not (last and j == CPS - 1)
            cur, nxt = sbuf[j % 2], sbuf[(j + 1) % 2]
            if has_next:
                prep_q(ci + 1)
            mx = l = acc = None
            toks = []
            for kt in range(NKT):
                if has_next:
                    mx = qk_piece(ci + 1, kt, nxt, mx)
                    toks.append(mx)
                tok = toks[kt - TIE_LAG][0:1] if (has_next and kt >= TIE_LAG) else None
                l, acc = sm_piece(ci, kt, cur, m, l, acc, tok)
                if kt == NKT - 1:
                    a_finish(ci, l, acc)
                    if has_next:
                        m = jnp.max(mx, axis=0, keepdims=True)
                yield m

    starts = {
        0: [xa_copy(1)],
        1: [xa_copy(2), xa_copy(3)] + group(0),
        2: wq_halves + group(1),
        4: wv_halves + group(2),
        6: group(3) + [wo_copy(0)],
        8: group(4) + [wo_copy(1)],
        10: [mem_copy, xb_head] + [wo_copy(n) for n in range(2, 8)],
        12: [xb_rest] + [xb_copy(c) for c in range(1, NRB)] + [awo_copy],
    }
    fences = sorted(starts)
    waits = {b: starts[a] for a, b in zip(fences[:-1], fences[1:])}
    retile_at = {2: (0, 2), 4: (1, 2), 6: (2, 2), 8: (3, 2), 10: (4, 2)}

    for c in (wk_a, xa_copy(0), wk_b):
        c.start()
    wk_a.wait()
    xa_copy(0).wait()
    side, side_left, pieces_left = iter(()), 0, 0
    for p in range(3 * NRB + 1):
        for c in waits.get(p, ()):
            c.wait()
        for c in starts.get(p, ()):
            c.start()
        if p == 3 * NRB:
            break
        if p == 0:
            for r in range(0, RB, PM):
                for g in range(WKA // 128):
                    proj_dot(xa[r:r + PM, :], r, 1, g, k4, None)
            wk_b.wait()
            for r in range(0, RB, PM):
                for g in range(WKA // 128, 8):
                    proj_dot(xa[r:r + PM, :], r, 1, g, k4, None)
            continue
        if p in retile_at:
            g, pieces_left = retile_at[p]
            side, side_left = retile(g), GROUPS[g] * D // RSUB
        n_side = side_left // pieces_left if pieces_left else 0
        side_left -= n_side
        pieces_left = max(pieces_left - 1, 0)
        j, rb = divmod(p, NRB)
        if j == 0:
            main, n_main = proj_rows(rb, 1, k4, None), 8 * RB // PM
        elif j == 1:
            main, n_main = proj_rows(rb, 0, q4, (DHA ** -0.5) * LOG2E), 8 * RB // PM
        else:
            main, n_main = proj_vt(rb), (RB // 128) * (D // TM)
        done = 0
        for i in range(n_main):
            next(main)
            while done < (i + 1) * n_side // n_main:
                next(side)
                done += 1
        if p == 2 * NRB - 1:
            prep_q(0)
            mx = None
            for kt in range(NKT):
                mx = qk_piece(0, kt, sbuf[0], mx)
            m0 = jnp.max(mx, axis=0, keepdims=True)
    assert side_left == 0
    pending.clear()

    row = lax.broadcasted_iota(i32, (L, L), 0)
    col = lax.broadcasted_iota(i32, (L, L), 1)
    mask = (row < M) | (row >= col)
    cb = (DHB ** -0.5) * LOG2E

    def step(s, m, last=False):
        r0 = s * SEG if isinstance(s, int) else pl.multiple_of(s * SEG, SEG)
        h_ref[M:L, :] = xb[pl.ds(r0, SEG), :].astype(f32)
        q0 = M if last else 0
        gen = a_pieces(s, m, last)
        npieces = CPS * NKT
        state = dict(done=0, m=m)
        heads = {}
        o_early = []

        def a_upto(n):
            while state["done"] < min(npieces, n):
                state["m"] = next(gen)
                state["done"] += 1

        def p1(t, j):
            hs = h_ref[q0:L, :] if j == 0 else h_ref[...]
            return jnp.dot(hs, _upk(wp[j * HB + t]), preferred_element_type=f32)

        def scores(t):
            e = heads[t]
            sc = lax.dot_general(e["q"], e["k"], (((1,), (1,)), ((), ())), preferred_element_type=f32)
            sc = jnp.where(mask[q0:L], sc, -1e9 * LOG2E)
            p = jnp.exp2(sc - jnp.max(sc, axis=1, keepdims=True))
            e["p"] = p
            e["r"] = _recip(jnp.sum(p, axis=1, keepdims=True))

        def attend(t):
            e = heads.pop(t)
            o_ref[q0:L, t * DHB:(t + 1) * DHB] = jnp.dot(e["p"], e["v"], preferred_element_type=f32) * e["r"]

        def p3_early(n):
            if not o_early:
                o_early.append(o_ref[q0:L, :KSPLIT])
            part_ref[n, q0:L] = jnp.dot(o_early[0], _upk(wop[n, :KSPLIT // 2, :]), preferred_element_type=f32)

        for t in range(NSLOT):
            base = state["done"]
            target = (t + 1) * npieces // ASLOTS
            if t < HB:
                e = heads[t] = {}
                e["q"] = p1(t, 0) * cb
                a_upto(base + int(round((target - base) / 2)))
                e["k"] = p1(t, 1).astype(bf16)
                e["v"] = p1(t, 2).astype(bf16)
                a_upto(target)
            if 0 <= t - D1 < HB:
                scores(t - D1)
            if t >= HB:
                a_upto(target)
            if 0 <= t - D1 - D2 < HB:
                attend(t - D1 - D2)
            for n in P3A_AT.get(t, ()):
                p3_early(n)
        o_late = o_ref[q0:L, KSPLIT:]
        for n in range(8):
            r = part_ref[n, q0:L] + jnp.dot(o_late, _upk(wop[n, KSPLIT // 2:, :]), preferred_element_type=f32)
            ob = r.astype(bf16)
            if last:
                xb[pl.ds(r0, SEG), n * 128:(n + 1) * 128] = ob
            else:
                xb[pl.ds(r0, SEG), n * 128:(n + 1) * 128] = ob[M:L]
                h_ref[0:M, n * 128:(n + 1) * 128] = ob[0:M].astype(f32)
        a_upto(npieces)
        if not last:
            ob_copy(r0).start()
        return state["m"]

    h_ref[0:M, :] = mem0v[...].astype(f32)
    spc = RB // SEG

    def two_steps(i, m):
        @pl.when(i == 1)
        def _():
            xb_rest.wait()

        @pl.when((i % (spc // 2) == 0) & (i > 0))
        def _():
            c = i // (spc // 2)
            c0 = pl.multiple_of(c * RB, RB)
            pltpu.make_async_copy(bx_hbm.at[pl.ds(c0, RB), :], xb.at[pl.ds(c0, RB), :], sem_xb.at[c]).wait()
        return step(2 * i + 1, step(2 * i, m))

    m_fin = lax.fori_loop(0, NSEG // 2 - 1, two_steps, m0)
    m_fin = step(NSEG - 2, m_fin)
    awo_copy.wait()
    step(NSEG - 1, m_fin, last=True)

    ooff = [sum(OBLOCKS[:i]) for i in range(len(OBLOCKS))]

    def oa_copy(i):
        return pltpu.make_async_copy(xa.at[pl.ds(ooff[i], OBLOCKS[i]), :],
                                     out_hbm.at[pl.ds(ooff[i], OBLOCKS[i]), pl.ds(0, D)], sem_oa.at[i])

    for i, (r0, nr) in enumerate(zip(ooff, OBLOCKS)):
        o_t = _upk(ot[:, r0:r0 + nr])
        y = lax.dot_general(o_t, awo[...], (((0,), (0,)), ((), ())), preferred_element_type=f32)
        xa[r0:r0 + nr, :] = y.astype(bf16)
        oa_copy(i).start()
        if i == 0:
            ob_copy((NSEG - 1) * SEG).start()
    for i in range(len(OBLOCKS)):
        oa_copy(i).wait()
    pltpu.make_async_copy(xb, out_hbm.at[:, pl.ds(D, D)], sem_ob).wait()


@functools.partial(jax.jit, static_argnames=("B_seg_len",))
def pallas_concat_heads__softmax_full_mha__memory_aug_recurrent_mem_tr__prompt_kernel(
    A_x: jax.Array,
    A_wqkv: jax.Array,
    A_wo: jax.Array,
    B_x: jax.Array,
    B_mem0: jax.Array,
    B_Wq: jax.Array,
    B_Wk: jax.Array,
    B_Wv: jax.Array,
    B_Wo: jax.Array,
    B_seg_len: int = SEG,
):
    assert A_x.shape == (1, S, D) and B_x.shape == (1, S, D) and B_mem0.shape == (1, M, D)
    assert A_wqkv.shape == (D, 3 * D) and A_wo.shape == (D, D)
    assert B_Wq.shape == B_Wk.shape == B_Wv.shape == (D, HB, DHB) and B_Wo.shape == (HB, DHB, D)
    assert int(B_seg_len) == SEG

    dma_sems = lambda n: pltpu.SemaphoreType.DMA((n,))
    scratch = [
        pltpu.VMEM((S, D), bf16),
        pltpu.VMEM((D, 3 * D), bf16),
        pltpu.VMEM((D, D), bf16),
        pltpu.VMEM((D, D), bf16),
        pltpu.VMEM((8, S // 2, 128), u32),
        pltpu.VMEM((8, S // 2, 128), u32),
        pltpu.VMEM((D // 2, S), u32),
        pltpu.VMEM((D // 2, S), u32),
        pltpu.VMEM((NQ // 2, 128), u32),
        pltpu.VMEM((S, D), bf16),
        pltpu.VMEM((M, D), bf16),
        pltpu.VMEM((NSTAGE, D, 128), u32),
        pltpu.VMEM((3 * HB, D // 2, 128), u32),
        pltpu.VMEM((8, HB * DHB // 2, 128), u32),
        pltpu.VMEM((L, D), f32),
        pltpu.VMEM((L, HB * DHB), f32),
        pltpu.VMEM((8, L, 128), f32),
        dma_sems(NRB), dma_sems(6), dma_sems(8), dma_sems(NRB), dma_sems(3), dma_sems(NSTAGE),
        dma_sems(len(OBLOCKS)), pltpu.SemaphoreType.DMA,
    ] + [pltpu.VMEM((KT, NQ), f32)] * (2 * NKT)

    out = pl.pallas_call(
        _kernel,
        out_shape=jax.ShapeDtypeStruct((S, 2 * D), bf16),
        in_specs=[pl.BlockSpec(memory_space=pl.ANY)] * 9,
        out_specs=pl.BlockSpec(memory_space=pl.ANY),
        scratch_shapes=scratch,
        compiler_params=pltpu.CompilerParams(vmem_limit_bytes=112 * 1024 * 1024),
    )(A_x.reshape(S, D), A_wqkv, A_wo, B_x.reshape(S, D), B_mem0.reshape(M, D), B_Wq, B_Wk, B_Wv,
      B_Wo.reshape(HB * DHB, D))
    return out.reshape(1, S, 2 * D)
```
